```python
import jax
import jax.numpy as jnp

def _softmax(x, axis=-1):
    return jax.nn.softmax(x, axis=axis)
def _gelu(x):
    return jax.nn.gelu(x, approximate=True)
def _silu(x):
    return jax.nn.silu(x)
def _sigmoid(x):
    return jax.nn.sigmoid(x)
def _layernorm(x, axis=-1, eps=1e-5):
    m = jnp.mean(x, axis=axis, keepdims=True)
    v = jnp.var(x, axis=axis, keepdims=True)
    return (x - m) / jnp.sqrt(v + eps)
def _scatter_add(tgt, idx, src, axis=0):
    return tgt.at[idx].add(src)
def _segment_sum(src, seg, n):
    return jax.ops.segment_sum(src, seg, n)
class _Rng:
    def __init__(self, key):
        self._k = key
    def _next(self):
        self._k, sub = jax.random.split(self._k)
        return sub
    def normal(self, shape):
        return jax.random.normal(self._next(), shape, dtype=jnp.bfloat16)
    def randint(self, lo, hi, shape):
        return jax.random.randint(self._next(), shape, lo, hi, dtype=jnp.int32)
    def uniform(self, shape, lo=0.0, hi=1.0):
        return jax.random.uniform(self._next(), shape, jnp.bfloat16, lo, hi)
    def permutation(self, n):
        return jax.random.permutation(self._next(), n)


kernel_name = 'recurrent_scan__sliding_local_dilated__glu_gated_swiglu__prompt'

def setup_inputs():
    _rng = _Rng(jax.random.key(int.from_bytes(__import__("os").urandom(4), "little")))
    _w = (lambda a: (lambda t: t.astype(jnp.bfloat16) if jnp.issubdtype(t.dtype, jnp.floating) else t)(jnp.asarray(a)))
    def _A_setup():
        B, S, D = 1, 2048, 1024
        return {
            "x": _w((lambda *s: _rng.normal(s) * 0.05)(B, S, D)),
            "wqkv": _w((lambda *s: _rng.normal(s) * 0.05)(D, 3 * D)),
            "wo": _w((lambda *s: _rng.normal(s) * 0.05)(D, D)),
        }
    _A_in = _A_setup()

    def _B_setup():
        B, S, D, F = 1, 2048, 1024, 3584
        return {
            "x": _w((lambda *s: _rng.normal(s) * 0.05)(B, S, D)),
            "w1": _w((lambda *s: _rng.normal(s) * 0.05)(D, F) * (2.0 / D) ** 0.5),
            "w3": _w((lambda *s: _rng.normal(s) * 0.05)(D, F) * (2.0 / D) ** 0.5),
            "w2": _w((lambda *s: _rng.normal(s) * 0.05)(F, D) * (2.0 / F) ** 0.5),
        }
    _B_in = _B_setup()

    return {
        "A_x": _A_in["x"],
        "A_wqkv": _A_in["wqkv"],
        "A_wo": _A_in["wo"],
        "B_x": _B_in["x"],
        "B_w1": _B_in["w1"],
        "B_w3": _B_in["w3"],
        "B_w2": _B_in["w2"],
    }

def reference(A_x, A_wqkv, A_wo, B_x, B_w1, B_w3, B_w2):
    def _A_ref(x, wqkv, wo):
        B, S, D = x.shape
        H = 32; Dh = D // H
        W, dil = 8, 2
        qkv = (lambda x, *d: x.transpose(*d))((x @ wqkv).reshape(B, S, 3, H, Dh), 2, 0, 3, 1, 4)
        q, k, v = qkv[0], qkv[1], qkv[2]
        scale = Dh ** -0.5
        pos = jnp.arange(S)
        off = jnp.arange(W) * dil
        idx = pos[:, None] - off[None, :]
        mask = idx >= 0
        idx_c = jnp.where(mask, idx, 0).reshape(-1)
        kg = k[:, :, idx_c, :].reshape(B, H, S, W, Dh)
        vg = v[:, :, idx_c, :].reshape(B, H, S, W, Dh)
        logits = jnp.einsum("bhsd,bhswd->bhsw", q, kg) * scale
        logits = jnp.where(mask[None, None, :, :], logits, -1e9)
        attn = _softmax(logits, axis=-1)
        o = jnp.einsum("bhsw,bhswd->bhsd", attn, vg)
        return (lambda x, *d: x.transpose(*d))(o, 0, 2, 1, 3).reshape(B, S, D) @ wo

    def _B_ref(x, w1, w3, w2):
        gate = jnp.einsum("bsd,df->bsf", x, w1)
        up = jnp.einsum("bsd,df->bsf", x, w3)
        h = _silu(gate) * up
        out = jnp.einsum("bsf,fd->bsd", h, w2)
        return out

    x = A_x
    xn = _layernorm(x, axis=-1)
    s = _A_ref(xn, A_wqkv, A_wo)
    g = _silu(_B_ref(xn, B_w1, B_w3, B_w2))
    return x + s * g
```

```python
import functools
import jax
import jax.numpy as jnp
from jax import lax
from jax.experimental import pallas as pl
from jax.experimental.pallas import tpu as pltpu

S, D, F = 2048, 1024, 3584
H, DH, W, DIL = 32, 32, 8, 2
TM = 512
NRB = S // TM
TF = 512
NC = F // TF
PAD = 16
NJ = D // 128
f32, bf16, u32 = jnp.float32, jnp.bfloat16, jnp.uint32


def _kernel(x_hbm, wqkv_hbm, wo_hbm, w1_hbm, w3_hbm, w2_hbm, out_hbm,
            x_v, xn_v, w1_v, w3_v, w2_v, wqkv_v, wt_v, wo_v, wop_v, acc_v,
            q_v, k_v, v_v, o_v, s_v, out_v,
            sem_x, sem_w1, sem_w3, sem_w2, sem_qkv, sem_wo, sem_out):

    def cp_x(rb):
        return pltpu.make_async_copy(x_hbm.at[pl.ds(rb * TM, TM)], x_v.at[pl.ds(rb * TM, TM)], sem_x.at[rb])

    def cp_w1(c):
        return pltpu.make_async_copy(w1_hbm.at[:, pl.ds(c * TF, TF)], w1_v.at[c], sem_w1.at[c])

    def cp_w3(c):
        return pltpu.make_async_copy(w3_hbm.at[:, pl.ds(c * TF, TF)], w3_v.at[c], sem_w3.at[c])

    def cp_w2(c):
        return pltpu.make_async_copy(w2_hbm.at[pl.ds(c * TF, TF)], w2_v.at[c], sem_w2.at[c])

    def cp_qkv():
        return pltpu.make_async_copy(wqkv_hbm, wqkv_v, sem_qkv)

    def cp_wo():
        return pltpu.make_async_copy(wo_hbm, wo_v, sem_wo)

    def cp_out(rb):
        r = pl.multiple_of(rb * TM, TM)
        return pltpu.make_async_copy(out_v.at[pl.ds(r, TM)], out_hbm.at[pl.ds(r, TM)], sem_out.at[rb])

    cp_x(0).start()
    cp_w1(0).start()
    cp_w3(0).start()
    cp_w2(0).start()
    for rb in range(1, NRB):
        cp_x(rb).start()
    cp_qkv().start()
    for c in range(1, NC):
        cp_w1(c).start()
        cp_w3(c).start()
        cp_w2(c).start()
        if c == 2:
            cp_wo().start()

    def layernorm(r0):
        x = x_v[pl.ds(r0, TM), :].astype(f32)
        m = jnp.mean(x, axis=-1, keepdims=True)
        xc = x - m
        v = jnp.mean(xc * xc, axis=-1, keepdims=True)
        xn_v[pl.ds(r0, TM), :] = (xc * lax.rsqrt(v + 1e-5)).astype(bf16)

    def ffn_h(r0, c):
        xn = xn_v[pl.ds(r0, TM), :]
        g = jnp.dot(xn, w1_v[c], preferred_element_type=f32)
        u = jnp.dot(xn, w3_v[c], preferred_element_type=f32)
        hg = 0.5 * g
        a = hg * u
        h = a + a * jnp.tanh(hg)
        return jnp.dot(h.astype(bf16), w2_v[c], preferred_element_type=f32)

    def wt_prep(cb):
        sec, h0 = cb // 8, (cb % 8) * 4
        for kb in range(NJ):
            t = pltpu.bitcast(wqkv_v[pl.ds(kb * 128, 128), pl.ds(cb * 128, 128)].T, u32)
            for hh in range(4):
                wt_v[kb, pl.ds(sec * 512 + h0 + hh, 16, stride=32), :] = t[hh * 16:(hh + 1) * 16, :]

    def wo_prep():
        for nb in range(NJ):
            t = pltpu.bitcast(wo_v[:, pl.ds(nb * 128, 128)], u32)
            for h in range(H):
                wop_v[nb, pl.ds(h, 16, stride=32), :] = t[h * 16:(h + 1) * 16, :]

    def qkv(r0):
        xn = xn_v[pl.ds(r0, TM), :]
        for sec in range(3):
            wt = jnp.concatenate([pltpu.bitcast(wt_v[kb, pl.ds(sec * 512, 512), :], bf16)
                                  for kb in range(NJ)], axis=1)
            r = lax.dot_general(xn, wt, (((1,), (1,)), ((), ())), preferred_element_type=f32)
            for j in range(NJ):
                blk = r[:, j * 128:(j + 1) * 128]
                if sec == 0:
                    q_v[j, pl.ds(r0, TM), :] = blk
                elif sec == 1:
                    k_v[j, pl.ds(r0 + PAD, TM), :] = blk
                else:
                    v_v[j, pl.ds(r0 + PAD, TM), :] = blk

    def attention(r0, rows):
        scale = DH ** -0.5
        lane = lax.broadcasted_iota(jnp.int32, (16, 128), 1)
        even = (lane & 1) == 0
        sub = lax.broadcasted_iota(jnp.int32, (16, 128), 0)
        for g in range(rows // 16):
            r = r0 + g * 16
            q = [q_v[j, pl.ds(r, 16), :] for j in range(NJ)]
            pos = sub + r
            L = []
            for w in range(W):
                p = q[0] * k_v[0, pl.ds(r + PAD - DIL * w, 16), :]
                for j in range(1, NJ):
                    p = p + q[j] * k_v[j, pl.ds(r + PAD - DIL * w, 16), :]
                p = p + pltpu.roll(p, 64, 1)
                p = p + jnp.where(even, pltpu.roll(p, 127, 1), pltpu.roll(p, 1, 1))
                p = p * scale
                if w > 0:
                    p = jnp.where(pos >= DIL * w, p, -1e9)
                L.append(p)
            m = L[0]
            for w in range(1, W):
                m = jnp.maximum(m, L[w])
            E = [jnp.exp(l - m) for l in L]
            den = E[0]
            for w in range(1, W):
                den = den + E[w]
            inv = 1.0 / den
            A = [e * inv for e in E]
            for j in range(NJ):
                o = A[0] * v_v[j, pl.ds(r + PAD, 16), :]
                for w in range(1, W):
                    o = o + A[w] * v_v[j, pl.ds(r + PAD - DIL * w, 16), :]
                o_v[pl.ds(r, 16), pl.ds(j * 128, 128)] = o.astype(bf16)

    def wo_mm(r0):
        wop = jnp.concatenate([pltpu.bitcast(wop_v[nb], bf16) for nb in range(NJ)], axis=1)
        s_v[pl.ds(r0, TM), :] = jnp.dot(o_v[pl.ds(r0, TM), :], wop, preferred_element_type=f32)

    def epilogue(r0, ffn):
        hg = 0.5 * ffn
        g = hg + hg * jnp.tanh(hg)
        out_v[pl.ds(r0, TM), :] = (x_v[pl.ds(r0, TM), :].astype(f32) + s_v[pl.ds(r0, TM), :] * g).astype(bf16)

    zpad = jnp.zeros((PAD, 128), f32)
    for j in range(NJ):
        k_v[j, pl.ds(0, PAD), :] = zpad
        v_v[j, pl.ds(0, PAD), :] = zpad

    def stage0(rb, _):
        r0 = pl.multiple_of(rb * TM, TM)
        cp_x(rb).wait()
        layernorm(r0)
        return 0
    lax.fori_loop(0, NRB, stage0, 0)

    def ffn_stage(c, rb, first, last):
        r0 = pl.multiple_of(rb * TM, TM)
        y = ffn_h(r0, c)
        if first:
            acc_v[pl.ds(r0, TM), :] = y
        elif last:
            epilogue(r0, acc_v[pl.ds(r0, TM), :] + y)
        else:
            acc_v[pl.ds(r0, TM), :] += y

    def wait_w(c):
        cp_w1(c).wait()
        cp_w3(c).wait()
        cp_w2(c).wait()

    wait_w(0)
    lax.fori_loop(0, NRB, lambda rb, _: (ffn_stage(0, rb, True, False), 0)[1], 0)

    cp_qkv().wait()
    for cb in range(24):
        wt_prep(cb)

    def st_qkv(rb, _):
        qkv(pl.multiple_of(rb * TM, TM))
        return 0
    lax.fori_loop(0, NRB, st_qkv, 0)

    def st_att(i, _):
        attention(pl.multiple_of(i * 128, 128), 128)
        return 0
    lax.fori_loop(0, S // 128, st_att, 0)

    def st_mid(c, _):
        wait_w(c)
        lax.fori_loop(0, NRB, lambda rb, _: (ffn_stage(c, rb, False, False), 0)[1], 0)
        return 0
    lax.fori_loop(1, NC - 1, st_mid, 0)

    cp_wo().wait()
    wo_prep()

    def st_wo(rb, _):
        wo_mm(pl.multiple_of(rb * TM, TM))
        return 0
    lax.fori_loop(0, NRB, st_wo, 0)

    wait_w(NC - 1)

    def st_last(rb, _):
        ffn_stage(NC - 1, rb, False, True)
        cp_out(rb).start()
        return 0
    lax.fori_loop(0, NRB, st_last, 0)
    for rb in range(NRB):
        cp_out(rb).wait()


@jax.jit
def pallas_recurrent_scan__sliding_local_dilated__glu_gated_swiglu__prompt_kernel(
    A_x: jax.Array,
    A_wqkv: jax.Array,
    A_wo: jax.Array,
    B_x: jax.Array,
    B_w1: jax.Array,
    B_w3: jax.Array,
    B_w2: jax.Array,
):
    del B_x
    x = A_x.reshape(S, D)
    V = pltpu.VMEM
    DMA = pltpu.SemaphoreType.DMA
    out = pl.pallas_call(
        _kernel,
        out_shape=jax.ShapeDtypeStruct((S, D), bf16),
        in_specs=[pl.BlockSpec(memory_space=pl.ANY)] * 6,
        out_specs=pl.BlockSpec(memory_space=pl.ANY),
        scratch_shapes=[
            V((S, D), bf16), V((S, D), bf16),
            V((NC, D, TF), bf16), V((NC, D, TF), bf16), V((NC, TF, D), bf16),
            V((D, 3 * D), bf16), V((NJ, 3 * D // 2, 128), u32),
            V((D, D), bf16), V((NJ, D // 2, 128), u32),
            V((S, D), f32),
            V((NJ, S, 128), f32), V((NJ, S + PAD, 128), f32), V((NJ, S + PAD, 128), f32),
            V((S, D), bf16), V((S, D), f32), V((S, D), bf16),
            DMA((NRB,)), DMA((NC,)), DMA((NC,)), DMA((NC,)), DMA(()), DMA(()), DMA((NRB,)),
        ],
        compiler_params=pltpu.CompilerParams(vmem_limit_bytes=120 * 1024 * 1024),
    )(x, A_wqkv, A_wo, B_w1, B_w3, B_w2)
    return out.reshape(1, S, D)
```

```python
import jax
import jax.numpy as jnp
from jax import lax
from jax.experimental import pallas as pl
from jax.experimental.pallas import tpu as pltpu

S, D, F = 2048, 1024, 3584
H, DH, W, DIL = 32, 32, 8, 2
TM = 512
NRB = S // TM
TB = 512
NB = S // TB
TF = 896
NC = F // TF
SUBS = (0, 256, 512, 896)
PAD = 16
NJ = D // 128
PITCH = 33
f32, bf16, u32 = jnp.float32, jnp.bfloat16, jnp.uint32


def _kernel(x_hbm, wqkv_hbm, wo_hbm, w1_hbm, w3_hbm, w2_hbm, out_hbm,
            x_v, xn_v, w1_v, w3_v, w2_v, wqkv_v, wt_v, wo_v, wop_v, acc_v,
            q_v, k_v, v_v, o_v, out_v,
            sem_x, sem_w, sem_s, sem_qkv, sem_wo, sem_out):

    def cp_x(rb):
        return [pltpu.make_async_copy(x_hbm.at[pl.ds(rb * TM, TM), pl.ds(j * 128, 128)],
                                      x_v.at[rb, j], sem_x.at[rb]) for j in range(NJ)]

    def cp_cols(a, n, sems):
        grp = [[pltpu.make_async_copy(src.at[:, pl.ds(j * 128, 128)], dst.at[j], sem)
                for j in range(a // 128, (a + n) // 128)]
               for src, dst, sem in ((w1_hbm, w1_v, sems[0]), (w3_hbm, w3_v, sems[1]))]
        grp.append([pltpu.make_async_copy(w2_hbm.at[pl.ds(a, n), pl.ds(j * 128, 128)],
                                          w2_v.at[a // TF, j, pl.ds(a % TF, n)], sems[2])
                    for j in range(NJ)])
        return grp

    def cp_w(c):
        return sum(cp_cols(c * TF, TF, [sem_w.at[i, c] for i in range(3)]), [])

    def cp_sub(s):
        return cp_cols(SUBS[s], SUBS[s + 1] - SUBS[s], [sem_s.at[i, s] for i in range(3)])

    def cp_qkv():
        return pltpu.make_async_copy(wqkv_hbm, wqkv_v, sem_qkv)

    def cp_wo():
        return [pltpu.make_async_copy(wo_hbm.at[:, pl.ds(j * 128, 128)], wo_v.at[j], sem_wo) for j in range(NJ)]

    def cp_out(rb, j0=0, nj=NJ):
        r = pl.multiple_of(rb * TM, TM)
        return [pltpu.make_async_copy(out_v.at[rb, j0 + j],
                                      out_hbm.at[pl.ds(r, TM), pl.ds(pl.multiple_of((j0 + j) * 128, 128), 128)],
                                      sem_out.at[rb]) for j in range(nj)]

    def start(cps):
        for cp in cps:
            cp.start()

    def wait(cps):
        for cp in cps:
            cp.wait()

    def layernorm(rb):
        for g in range(TM // 16):
            xs = [x_v[rb, j, pl.ds(g * 16, 16), :].astype(f32) for j in range(NJ)]
            t = xs[0]
            for j in range(1, NJ):
                t = t + xs[j]
            m = jnp.sum(t, axis=-1, keepdims=True) * (1.0 / D)
            xc = [x - m for x in xs]
            t = xc[0] * xc[0]
            for j in range(1, NJ):
                t = t + xc[j] * xc[j]
            v = jnp.sum(t, axis=-1, keepdims=True) * (1.0 / D)
            rs = lax.rsqrt(v + 1e-5)
            for j in range(NJ):
                xn_v[rb, j, pl.ds(g * 16, 16), :] = (xc[j] * rs).astype(bf16)

    def packed(ref):
        return pltpu.bitcast(ref.bitcast(u32)[...], bf16)

    def wide(ref, i):
        return jnp.concatenate([ref[i, j] for j in range(NJ)], axis=1)

    def ffn(rb, c, a=0, n=TF, first=False, waits=None):
        rows = pl.ds(pl.multiple_of(rb * TM, TM), TM)
        if not first:
            y = acc_v[rows, :]
        xn = wide(xn_v, rb)
        j0 = c * (TF // 128) + a // 128
        if waits:
            wait(waits[0])
        w1 = jnp.concatenate([packed(w1_v.at[j0 + j]) for j in range(n // 128)], axis=1)
        g = jnp.dot(xn, w1, preferred_element_type=f32)
        if waits:
            wait(waits[1])
        w3 = jnp.concatenate([packed(w3_v.at[j0 + j]) for j in range(n // 128)], axis=1)
        u = jnp.dot(xn, w3, preferred_element_type=f32)
        hg = 0.5 * g
        t = hg * u
        h = t + t * jnp.tanh(hg)
        if waits:
            wait(waits[2])
        if n == TF:
            w2 = jnp.concatenate([packed(w2_v.at[c, j]) for j in range(NJ)], axis=1)
        else:
            w2 = jnp.concatenate([packed(w2_v.at[c, j, pl.ds(a, n)]) for j in range(NJ)], axis=1)
        d = jnp.dot(h.astype(bf16), w2, preferred_element_type=f32)
        acc_v[rows, :] = d if first else y + d

    def wt_prep(cb):
        sec, h0 = cb // 8, (cb % 8) * 4
        for kb in range(NJ):
            t = pltpu.bitcast(wqkv_v[pl.ds(kb * 128, 128), pl.ds(pl.multiple_of(cb * 128, 128), 128)].T, u32)
            for hh in range(4):
                wt_v[kb, pl.ds(sec * PITCH * 16 + h0 + hh, 16, stride=PITCH), :] = t[hh * 16:(hh + 1) * 16, :]

    def wo_prep(nb):
        t = wo_v.at[nb].bitcast(u32)[...]
        for h in range(H):
            wop_v[nb, pl.ds(h, 16, stride=PITCH), :] = t[h * 16:(h + 1) * 16, :]

    def qkv(rb):
        r0, m = pl.multiple_of(rb * TM, TM), TM
        xn = wide(xn_v, rb)
        for sec in range(3):
            wt = jnp.concatenate(
                [jnp.concatenate([pltpu.bitcast(wt_v[kb, pl.ds((sec * 16 + dd) * PITCH, 32), :], bf16)
                                  for dd in range(16)], axis=0)
                 for kb in range(NJ)], axis=1)
            r = lax.dot_general(xn, wt, (((1,), (1,)), ((), ())), preferred_element_type=f32)
            for j in range(NJ):
                blk = r[:, j * 128:(j + 1) * 128]
                if sec == 0:
                    q_v[j, pl.ds(r0, m), :] = blk
                elif sec == 1:
                    k_v[j, pl.ds(r0 + PAD, m), :] = blk
                else:
                    v_v[j, pl.ds(r0 + PAD, m), :] = blk

    def attention(r0, rows, masked=False):
        scale = DH ** -0.5
        lane = lax.broadcasted_iota(jnp.int32, (16, 128), 1)
        even = (lane & 1) == 0
        sub = lax.broadcasted_iota(jnp.int32, (16, 128), 0)
        for g in range(rows // 16):
            r = r0 + g * 16
            cache = {}

            def kw(ref, j, r, w, cache=cache):
                key = (id(ref), j, w % 4)
                if key not in cache:
                    cache[key] = ref[j, pl.ds(r + PAD - DIL * (w % 4) - 8, 24), :]
                return cache[key][8:24] if w < 4 else cache[key][0:16]

            q = [q_v[j, pl.ds(r, 16), :] for j in range(NJ)]
            pos = sub + r
            L = []
            for w in range(W):
                p = q[0] * kw(k_v, 0, r, w)
                for j in range(1, NJ):
                    p = p + q[j] * kw(k_v, j, r, w)
                p = p + pltpu.roll(p, 64, 1)
                p = p + jnp.where(even, pltpu.roll(p, 127, 1), pltpu.roll(p, 1, 1))
                if masked and w > 0:
                    p = jnp.where(sub + r >= DIL * w, p, -1e30)
                L.append(p)
            m = L[0]
            for w in range(1, W):
                m = jnp.maximum(m, L[w])
            E = [jnp.exp2((l - m) * (scale * 1.4426950408889634)) for l in L]
            den = E[0]
            for w in range(1, W):
                den = den + E[w]
            inv = pl.reciprocal(den, approx=True)
            inv = inv * (2.0 - den * inv)
            A = [e * inv for e in E]
            for j in range(NJ):
                o = A[0] * kw(v_v, j, r, 0)
                for w in range(1, W):
                    o = o + A[w] * kw(v_v, j, r, w)
                o_v[j, r // 16] = o.astype(bf16)

    def wo_mm(rb, j0=0, nj=NJ):
        rows = pl.ds(pl.multiple_of(rb * TM, TM), TM)
        cols = pl.ds(pl.multiple_of(j0 * 128, 128), nj * 128)
        y = acc_v[rows, cols]
        hg = 0.5 * y
        gate = hg + hg * jnp.tanh(hg)
        wop = jnp.concatenate(
            [jnp.concatenate([pltpu.bitcast(wop_v[j0 + nb, pl.ds(dd * PITCH, 32), :], bf16)
                              for dd in range(16)], axis=0)
             for nb in range(nj)], axis=1)
        o = jnp.concatenate([o_v[j, pl.ds(rb * (TM // 16), TM // 16)].reshape(TM, 128) for j in range(NJ)], axis=1)
        s = jnp.dot(o, wop, preferred_element_type=f32)
        for j in range(nj):
            c = slice(j * 128, (j + 1) * 128)
            out_v[rb, j0 + j] = (x_v[rb, j0 + j].astype(f32) + s[:, c] * gate[:, c]).astype(bf16)

    sub0 = cp_sub(0)
    start(cp_x(0))
    start(sub0[0])
    zpad = jnp.zeros((PAD, 128), f32)
    for j in range(NJ):
        k_v[j, pl.ds(0, PAD), :] = zpad
        v_v[j, pl.ds(0, PAD), :] = zpad
    wait(cp_x(0))
    start(sub0[1])
    start(sub0[2])
    layernorm(0)
    start(sum(cp_sub(1), []))

    ffn(0, 0, SUBS[0], SUBS[1] - SUBS[0], first=True, waits=sub0)
    wait(sum(cp_sub(1), []))
    start(cp_x(1))
    start(sum(cp_sub(2), []))
    ffn(0, 0, SUBS[1], SUBS[2] - SUBS[1])
    wait(cp_x(1))
    wait(sum(cp_sub(2), []))
    start(cp_x(2))
    start(cp_x(3))
    ffn(0, 0, SUBS[2], SUBS[3] - SUBS[2])
    layernorm(1)
    wait(cp_x(2))
    wait(cp_x(3))
    start(cp_wo())
    start(cp_w(1))
    cp_qkv().start()
    for rb in range(1, NRB):
        ffn(rb, 0, first=True)
        if rb < NRB - 1:
            layernorm(rb + 1)
    wait(cp_wo())
    for nb in range(NJ):
        wo_prep(nb)

    cp_qkv().wait()
    wait(cp_w(1))
    start(cp_w(2))

    def l2(i, _):
        ffn(i, 1)
        for t in range(24 // NB):
            wt_prep(i * (24 // NB) + t)
        return 0
    lax.fori_loop(0, NB, l2, 0)

    start(cp_w(3))

    def l3(i, _):
        qkv(i)
        return 0
    lax.fori_loop(0, NB, l3, 0)

    wait(cp_w(2))
    wait(cp_w(3))

    def l4(i, _):
        ffn(i % NB, 2 + i // NB)
        attention(pl.multiple_of(i * (TB // 2), TB // 2), TB // 2)
        return 0
    lax.fori_loop(0, 2 * NB, l4, 0)

    attention(0, 16, masked=True)

    def l6(rb, _):
        wo_mm(rb)
        start(cp_out(rb))
        return 0
    lax.fori_loop(0, NRB - 1, l6, 0)

    def l7(hf, _):
        wo_mm(NRB - 1, hf * (NJ // 2), NJ // 2)
        start(cp_out(NRB - 1, hf * (NJ // 2), NJ // 2))
        return 0
    lax.fori_loop(0, 2, l7, 0)
    for rb in range(NRB):
        wait(cp_out(rb))


@jax.jit
def pallas_recurrent_scan__sliding_local_dilated__glu_gated_swiglu__prompt_kernel(
    A_x: jax.Array,
    A_wqkv: jax.Array,
    A_wo: jax.Array,
    B_x: jax.Array,
    B_w1: jax.Array,
    B_w3: jax.Array,
    B_w2: jax.Array,
):
    del B_x
    x = A_x.reshape(S, D)
    V = pltpu.VMEM
    DMA = pltpu.SemaphoreType.DMA
    out = pl.pallas_call(
        _kernel,
        out_shape=jax.ShapeDtypeStruct((S, D), bf16),
        in_specs=[pl.BlockSpec(memory_space=pl.ANY)] * 6,
        out_specs=pl.BlockSpec(memory_space=pl.ANY),
        scratch_shapes=[
            V((NRB, NJ, TM, 128), bf16), V((NRB, NJ, TM, 128), bf16),
            V((F // 128, D, 128), bf16), V((F // 128, D, 128), bf16), V((NC, NJ, TF, 128), bf16),
            V((D, 3 * D), bf16), V((NJ, 3 * 16 * PITCH, 128), u32),
            V((NJ, D, 128), bf16), V((NJ, 16 * PITCH, 128), u32),
            V((S, D), f32),
            V((NJ, S, 128), f32), V((NJ, S + PAD, 128), f32), V((NJ, S + PAD, 128), f32),
            V((NJ, S // 16, 16, 128), bf16), V((NRB, NJ, TM, 128), bf16),
            DMA((NRB,)), DMA((3, NC)), DMA((3, 3)), DMA(()), DMA(()), DMA((NRB,)),
        ],
        compiler_params=pltpu.CompilerParams(vmem_limit_bytes=120 * 1024 * 1024),
    )(x, A_wqkv, A_wo, B_w1, B_w3, B_w2)
    return out.reshape(1, S, D)
```

```python
import jax
import jax.numpy as jnp
from jax import lax
from jax.experimental import pallas as pl
from jax.experimental.pallas import tpu as pltpu

S, D, F = 2048, 1024, 3584
H, DH, W, DIL = 32, 32, 8, 2
TM = 512
NRB = S // TM
TB = 512
NB = S // TB
TF = 896
NC = F // TF
SUBS = (0, 256, 512, 896)
PAD = 16
NJ = D // 128
PITCH = 33
LN_ROLL = True
LN_G = 32
WO_POS = 'l2'
ACC_EARLY = False
KW24 = False
TREE = False
NORM_O = False
BLOCKS = False
PK_X = True
PK_O = False
f32, bf16, u32 = jnp.float32, jnp.bfloat16, jnp.uint32


def _kernel(x_hbm, wqkv_hbm, wo_hbm, w1_hbm, w3_hbm, w2_hbm, out_hbm,
            x_v, xn_v, w1_v, w3_v, w2_v, wqkv_v, wt_v, wo_v, wop_v, acc_v,
            q_v, k_v, v_v, o_v, out_v,
            one_ref, sem_x, sem_w, sem_s, sem_qkv, sem_wo, sem_out):

    def cp_x(rb):
        return [pltpu.make_async_copy(x_hbm.at[pl.ds(rb * TM, TM), pl.ds(j * 128, 128)],
                                      x_v.at[rb, j], sem_x.at[rb]) for j in range(NJ)]

    def cp_cols(a, n, sems):
        grp = [[pltpu.make_async_copy(src.at[:, pl.ds(j * 128, 128)], dst.at[j], sem)
                for j in range(a // 128, (a + n) // 128)]
               for src, dst, sem in ((w1_hbm, w1_v, sems[0]), (w3_hbm, w3_v, sems[1]))]
        grp.append([pltpu.make_async_copy(w2_hbm.at[pl.ds(a, n), pl.ds(j * 128, 128)],
                                          w2_v.at[a // TF, j, pl.ds(a % TF, n)], sems[2])
                    for j in range(NJ)])
        return grp

    def cp_w(c):
        return sum(cp_cols(c * TF, TF, [sem_w.at[i, c] for i in range(3)]), [])

    def cp_sub(s):
        return cp_cols(SUBS[s], SUBS[s + 1] - SUBS[s], [sem_s.at[i, s] for i in range(3)])

    def cp_qkv():
        return pltpu.make_async_copy(wqkv_hbm, wqkv_v, sem_qkv)

    def cp_wo():
        return [pltpu.make_async_copy(wo_hbm.at[:, pl.ds(j * 128, 128)], wo_v.at[j], sem_wo) for j in range(NJ)]

    def cp_out(rb, j0=0, nj=NJ):
        r = pl.multiple_of(rb * TM, TM)
        return [pltpu.make_async_copy(out_v.at[rb, j0 + j],
                                      out_hbm.at[pl.ds(r, TM), pl.ds(pl.multiple_of((j0 + j) * 128, 128), 128)],
                                      sem_out.at[rb]) for j in range(nj)]

    def start(cps):
        for cp in cps:
            cp.start()

    def wait(cps):
        for cp in cps:
            cp.wait()

    def lane_sum(t, roll):
        if not roll:
            return jnp.sum(t, axis=-1, keepdims=True)
        for sh in (64, 32, 16, 8, 4, 2, 1):
            t = t + pltpu.roll(t, sh, 1)
        return t

    def layernorm(rb):
        roll = LN_ROLL and rb > 0
        for g in range(TM // LN_G):
            rows = pl.ds(g * LN_G, LN_G)
            if PK_X:
                x32 = x_v.at[rb].bitcast(u32)
                xs = []
                for j in range(NJ):
                    w32 = x32[j, pl.ds(g * (LN_G // 2), LN_G // 2), :]
                    xs.append(jnp.concatenate(
                        [pltpu.unpack_elementwise(w32, index=i, packed_dtype=bf16, unpacked_dtype=f32)
                         for i in range(2)], axis=0))
            else:
                xs = [x_v[rb, j, rows, :].astype(f32) for j in range(NJ)]
            t = xs[0]
            for j in range(1, NJ):
                t = t + xs[j]
            m = lane_sum(t, roll) * (1.0 / D)
            xc = [x - m for x in xs]
            t = xc[0] * xc[0]
            for j in range(1, NJ):
                t = t + xc[j] * xc[j]
            v = lane_sum(t, roll) * (1.0 / D)
            rs = lax.rsqrt(v + 1e-5)
            for j in range(NJ):
                y = xc[j] * rs
                if PK_X:
                    xn_v[rb, j, pl.ds(g * (LN_G // 2), LN_G // 2), :] = pltpu.pack_elementwise(
                        [y[:LN_G // 2], y[LN_G // 2:]], packed_dtype=bf16)
                else:
                    xn_v[rb, j, rows, :] = y.astype(bf16)

    def packed(ref):
        return pltpu.bitcast(ref.bitcast(u32)[...], bf16)

    def wide(ref, i):
        if PK_X:
            return jnp.concatenate([pltpu.bitcast(ref[i, j], bf16) for j in range(NJ)], axis=1)
        return jnp.concatenate([ref[i, j] for j in range(NJ)], axis=1)

    def ffn(rb, c, a=0, n=TF, first=False, waits=None, then=None):
        rows = pl.ds(pl.multiple_of(rb * TM, TM), TM)
        if not first and ACC_EARLY:
            y = acc_v[rows, :]
        xn = wide(xn_v, rb)
        j0 = c * (TF // 128) + a // 128
        if waits:
            wait(waits[0])
        w1 = jnp.concatenate([packed(w1_v.at[j0 + j]) for j in range(n // 128)], axis=1)
        g = jnp.dot(xn, w1, preferred_element_type=f32)
        if waits:
            wait(waits[1])
        w3 = jnp.concatenate([packed(w3_v.at[j0 + j]) for j in range(n // 128)], axis=1)
        u = jnp.dot(xn, w3, preferred_element_type=f32)
        hg = 0.5 * g
        t = hg * u
        h = t + t * jnp.tanh(hg)
        if waits:
            wait(waits[2])
            then()
        if n == TF:
            w2 = jnp.concatenate([packed(w2_v.at[c, j]) for j in range(NJ)], axis=1)
        else:
            w2 = jnp.concatenate([packed(w2_v.at[c, j, pl.ds(a, n)]) for j in range(NJ)], axis=1)
        d = jnp.dot(h.astype(bf16), w2, preferred_element_type=f32)
        acc_v[rows, :] = d if first else (y if ACC_EARLY else acc_v[rows, :]) + d

    def wt_prep(cb):
        sec, h0 = cb // 8, (cb % 8) * 4
        for kb in range(NJ):
            t = pltpu.bitcast(wqkv_v[pl.ds(kb * 128, 128), pl.ds(pl.multiple_of(cb * 128, 128), 128)].T, u32)
            for hh in range(4):
                wt_v[kb, pl.ds(sec * PITCH * 16 + h0 + hh, 16, stride=PITCH), :] = t[hh * 16:(hh + 1) * 16, :]

    def wo_prep(nb):
        t = wo_v.at[nb].bitcast(u32)[...]
        for h in range(H):
            wop_v[nb, pl.ds(h, 16, stride=PITCH), :] = t[h * 16:(h + 1) * 16, :]

    def qkv(rb):
        r0, m = pl.multiple_of(rb * TM, TM), TM
        xn = wide(xn_v, rb)
        for sec in range(3):
            wt = jnp.concatenate(
                [jnp.concatenate([pltpu.bitcast(wt_v[kb, pl.ds((sec * 16 + dd) * PITCH, 32), :], bf16)
                                  for dd in range(16)], axis=0)
                 for kb in range(NJ)], axis=1)
            r = lax.dot_general(xn, wt, (((1,), (1,)), ((), ())), preferred_element_type=f32)
            for j in range(NJ):
                blk = r[:, j * 128:(j + 1) * 128]
                if sec == 0:
                    q_v[j, pl.ds(r0, m), :] = blk
                elif sec == 1:
                    k_v[j, pl.ds(r0 + PAD, m), :] = blk
                else:
                    v_v[j, pl.ds(r0 + PAD, m), :] = blk

    def attention(r0, rows, masked=False):
        c = DH ** -0.5 * 1.4426950408889634
        lane = lax.broadcasted_iota(jnp.int32, (16, 128), 1)
        even = (lane & 1) == 0
        sub = lax.broadcasted_iota(jnp.int32, (16, 128), 0)
        if PK_O:
            sub = (sub & 7) * 2 + (sub >> 3)

        def total(t):
            if TREE:
                return ((t[0] + t[1]) + (t[2] + t[3])) + ((t[4] + t[5]) + (t[6] + t[7]))
            p = t[0]
            for x in t[1:]:
                p = p + x
            return p

        for g in range(rows // 16):
            r = r0 + g * 16
            cache = {}

            def kw(ref, j, w, r=r, cache=cache):
                if PK_O:
                    return jnp.concatenate([ref[j, pl.ds(r + PAD - DIL * w + p, 8, stride=2), :] for p in range(2)], axis=0)
                if not KW24:
                    return ref[j, pl.ds(r + PAD - DIL * w, 16), :]
                key = (id(ref), j, w % 4)
                if key not in cache:
                    cache[key] = ref[j, pl.ds(r + PAD - DIL * (w % 4) - 8, 24), :]
                return cache[key][8:24] if w < 4 else cache[key][0:16]

            if PK_O:
                q = [jnp.concatenate([q_v[j, pl.ds(r + p, 8, stride=2), :] for p in range(2)], axis=0) for j in range(NJ)]
            else:
                q = [q_v[j, pl.ds(r, 16), :] for j in range(NJ)]
            L = []
            for w in range(W):
                p = total([q[j] * kw(k_v, j, w) for j in range(NJ)])
                p = p + pltpu.roll(p, 64, 1)
                p = p + jnp.where(even, pltpu.roll(p, 127, 1), pltpu.roll(p, 1, 1))
                if masked and w > 0:
                    p = jnp.where(sub + r >= DIL * w, p, -1e30)
                L.append(p)
            m = L[0]
            for w in range(1, W):
                m = jnp.maximum(m, L[w])
            E = [jnp.exp2((l - m) * c) for l in L]
            den = total(E)
            inv = pl.reciprocal(den, approx=True)
            inv = inv * (2.0 - den * inv)
            A = E if NORM_O else [e * inv for e in E]
            for j in range(NJ):
                o = total([A[w] * kw(v_v, j, w) for w in range(W)])
                o = o * inv if NORM_O else o
                if PK_O:
                    o_v[j, r // 16] = pltpu.pack_elementwise([o[:8], o[8:]], packed_dtype=bf16)
                else:
                    o_v[j, r // 16] = o.astype(bf16)

    def wo_mm(rb, j0=0, nj=NJ):
        rows = pl.ds(pl.multiple_of(rb * TM, TM), TM)
        cols = pl.ds(pl.multiple_of(j0 * 128, 128), nj * 128)
        y = acc_v[rows, cols]
        hg = 0.5 * y
        gate = hg + hg * jnp.tanh(hg)
        wop = jnp.concatenate(
            [jnp.concatenate([pltpu.bitcast(wop_v[j0 + nb, pl.ds(dd * PITCH, 32), :], bf16)
                              for dd in range(16)], axis=0)
             for nb in range(nj)], axis=1)
        if PK_O:
            o = jnp.concatenate([pltpu.bitcast(o_v[j, pl.ds(rb * (TM // 16), TM // 16)].reshape(TM // 2, 128), bf16)
                                 for j in range(NJ)], axis=1)
        else:
            o = jnp.concatenate([o_v[j, pl.ds(rb * (TM // 16), TM // 16)].reshape(TM, 128) for j in range(NJ)], axis=1)
        s = jnp.dot(o, wop, preferred_element_type=f32)
        for j in range(nj):
            c = slice(j * 128, (j + 1) * 128)
            out_v[rb, j0 + j] = (x_v[rb, j0 + j].astype(f32) + s[:, c] * gate[:, c]).astype(bf16)

    sub0 = cp_sub(0)
    start(cp_x(0))
    start(sub0[0])
    zpad = jnp.zeros((PAD, 128), f32)
    for j in range(NJ):
        k_v[j, pl.ds(0, PAD), :] = zpad
        v_v[j, pl.ds(0, PAD), :] = zpad
    wait(cp_x(0))
    start(sub0[1])
    start(sub0[2])
    layernorm(0)
    start(sum(cp_sub(1), []))

    ffn(0, 0, SUBS[0], SUBS[1] - SUBS[0], first=True, waits=sub0,
        then=lambda: start(sum(cp_sub(2), [])))
    wait(sum(cp_sub(1), []))
    start(cp_x(1))
    ffn(0, 0, SUBS[1], SUBS[2] - SUBS[1])
    wait(cp_x(1))
    wait(sum(cp_sub(2), []))
    start(cp_x(2))
    start(cp_x(3))
    ffn(0, 0, SUBS[2], SUBS[3] - SUBS[2])
    layernorm(1)
    wait(cp_x(2))
    wait(cp_x(3))
    start(cp_wo())
    start(cp_w(1))
    cp_qkv().start()
    one_ref[0] = 1
    one = one_ref[0]

    def block(f):
        if BLOCKS:
            lax.fori_loop(0, one, lambda i, c: (f(), c)[1], 0)
        else:
            f()

    for rb in range(1, NRB):
        def unit(rb=rb):
            ffn(rb, 0, first=True)
            if rb < NRB - 1:
                layernorm(rb + 1)
        if rb == NRB - 1 and WO_POS == 'end':
            wait(cp_wo())

            def unit(rb=rb):
                ffn(rb, 0, first=True)
                for nb in range(NJ):
                    wo_prep(nb)
        block(unit)

    cp_qkv().wait()
    if WO_POS != 'end':
        wait(cp_wo())
    wait(cp_w(1))
    start(cp_w(2))

    def l2(i, _):
        ffn(i, 1)
        for t in range(24 // NB):
            wt_prep(i * (24 // NB) + t)
        if WO_POS == 'l2':
            wo_prep(2 * i)
            wo_prep(2 * i + 1)
        return 0
    lax.fori_loop(0, NB, l2, 0)

    start(cp_w(3))

    def l3(i, _):
        qkv(i)
        if WO_POS == 'l3':
            wo_prep(2 * i)
            wo_prep(2 * i + 1)
        return 0
    lax.fori_loop(0, NB, l3, 0)

    wait(cp_w(2))
    wait(cp_w(3))

    def l4(i, _):
        ffn(i % NB, 2 + i // NB)
        attention(pl.multiple_of(i * (TB // 2), TB // 2), TB // 2)
        if WO_POS == 'l4':
            wo_prep(i)
        return 0
    lax.fori_loop(0, 2 * NB, l4, 0)

    attention(0, 16, masked=True)

    def l6(rb, _):
        wo_mm(rb)
        start(cp_out(rb))
        return 0
    lax.fori_loop(0, NRB - 1, l6, 0)

    def l7(hf, _):
        wo_mm(NRB - 1, hf * (NJ // 2), NJ // 2)
        start(cp_out(NRB - 1, hf * (NJ // 2), NJ // 2))
        return 0
    lax.fori_loop(0, 2, l7, 0)
    for rb in range(NRB):
        wait(cp_out(rb))


@jax.jit
def pallas_recurrent_scan__sliding_local_dilated__glu_gated_swiglu__prompt_kernel(
    A_x: jax.Array,
    A_wqkv: jax.Array,
    A_wo: jax.Array,
    B_x: jax.Array,
    B_w1: jax.Array,
    B_w3: jax.Array,
    B_w2: jax.Array,
):
    del B_x
    x = A_x.reshape(S, D)
    V = pltpu.VMEM
    DMA = pltpu.SemaphoreType.DMA
    out = pl.pallas_call(
        _kernel,
        out_shape=jax.ShapeDtypeStruct((S, D), bf16),
        in_specs=[pl.BlockSpec(memory_space=pl.ANY)] * 6,
        out_specs=pl.BlockSpec(memory_space=pl.ANY),
        scratch_shapes=[
            V((NRB, NJ, TM, 128), bf16),
            V((NRB, NJ, TM // 2, 128), u32) if PK_X else V((NRB, NJ, TM, 128), bf16),
            V((F // 128, D, 128), bf16), V((F // 128, D, 128), bf16), V((NC, NJ, TF, 128), bf16),
            V((D, 3 * D), bf16), V((NJ, 3 * 16 * PITCH, 128), u32),
            V((NJ, D, 128), bf16), V((NJ, 16 * PITCH, 128), u32),
            V((S, D), f32),
            V((NJ, S, 128), f32), V((NJ, S + PAD, 128), f32), V((NJ, S + PAD, 128), f32),
            V((NJ, S // 16, 8, 128), u32) if PK_O else V((NJ, S // 16, 16, 128), bf16), V((NRB, NJ, TM, 128), bf16),
            pltpu.SMEM((1,), jnp.int32),
            DMA((NRB,)), DMA((3, NC)), DMA((3, 3)), DMA(()), DMA(()), DMA((NRB,)),
        ],
        compiler_params=pltpu.CompilerParams(vmem_limit_bytes=120 * 1024 * 1024),
    )(x, A_wqkv, A_wo, B_w1, B_w3, B_w2)
    return out.reshape(1, S, D)
```

```python
import jax
import jax.numpy as jnp
from jax import lax
from jax.experimental import pallas as pl
from jax.experimental.pallas import tpu as pltpu

S, D, F = 2048, 1024, 3584
H, DH, W, DIL = 32, 32, 8, 2
TM = 512
NRB = S // TM
TB = 512
NB = S // TB
TF = 896
NC = F // TF
SUBS = (0, 256, 512, 896)
PAD = 16
NJ = D // 128
PITCH = 33
LN_ROLL = True
LN_G = 32
WO_POS = 'l2'
ACC_EARLY = False
KW24 = True
TREE = False
NORM_O = False
BLOCKS = False
ONESTAGE = False
PRESCALE = False
RECIP = 'newton'
NOROLL = False
UPACK = True
PVROLL = 3
QKROLL = 0
LNROLL2 = 0
LNROLLX = 0
LN_NR = (0, 1, 3, 3)
PK_X = True
PK_O = False
f32, bf16, u32 = jnp.float32, jnp.bfloat16, jnp.uint32


def _kernel(x_hbm, wqkv_hbm, wo_hbm, w1_hbm, w3_hbm, w2_hbm, out_hbm,
            x_v, xn_v, w1_v, w3_v, w2_v, wqkv_v, wt_v, wo_v, wop_v, acc_v,
            q_v, k_v, v_v, o_v, out_v,
            one_ref, sem_x, sem_w, sem_s, sem_qkv, sem_wo, sem_out):

    def cp_x(rb):
        return [pltpu.make_async_copy(x_hbm.at[pl.ds(rb * TM, TM), pl.ds(j * 128, 128)],
                                      x_v.at[rb, j], sem_x.at[rb]) for j in range(NJ)]

    def cp_cols(a, n, sems):
        grp = [[pltpu.make_async_copy(src.at[:, pl.ds(j * 128, 128)], dst.at[j], sem)
                for j in range(a // 128, (a + n) // 128)]
               for src, dst, sem in ((w1_hbm, w1_v, sems[0]), (w3_hbm, w3_v, sems[1]))]
        grp.append([pltpu.make_async_copy(w2_hbm.at[pl.ds(a, n), pl.ds(j * 128, 128)],
                                          w2_v.at[a // TF, j, pl.ds(a % TF, n)], sems[2])
                    for j in range(NJ)])
        return grp

    def cp_w(c):
        return sum(cp_cols(c * TF, TF, [sem_w.at[i, c] for i in range(3)]), [])

    def cp_sub(s):
        return cp_cols(SUBS[s], SUBS[s + 1] - SUBS[s], [sem_s.at[i, s] for i in range(3)])

    def cp_qkv():
        return pltpu.make_async_copy(wqkv_hbm, wqkv_v, sem_qkv)

    def cp_wo():
        return [pltpu.make_async_copy(wo_hbm.at[:, pl.ds(j * 128, 128)], wo_v.at[j], sem_wo) for j in range(NJ)]

    def cp_out(rb, j0=0, nj=NJ):
        r = pl.multiple_of(rb * TM, TM)
        return [pltpu.make_async_copy(out_v.at[rb, j0 + j],
                                      out_hbm.at[pl.ds(r, TM), pl.ds(pl.multiple_of((j0 + j) * 128, 128), 128)],
                                      sem_out.at[rb]) for j in range(nj)]

    def start(cps):
        for cp in cps:
            cp.start()

    def wait(cps):
        for cp in cps:
            cp.wait()

    def lane_sum(t, nr):
        for sh in (64, 32, 16, 8, 4, 2, 1)[:nr]:
            t = t + pltpu.roll(t, sh, 1)
        if nr == 7:
            return t
        return jnp.sum(t, axis=-1, keepdims=True) * (0.5 ** nr)

    def layernorm(rb):
        roll = LN_NR[rb]
        for g in range(TM // LN_G):
            rows = pl.ds(g * LN_G, LN_G)
            if PK_X:
                x32 = x_v.at[rb].bitcast(u32)
                xs = []
                for j in range(NJ):
                    w32 = x32[j, pl.ds(g * (LN_G // 2), LN_G // 2), :]
                    xs.append(jnp.concatenate(
                        [pltpu.unpack_elementwise(w32, index=i, packed_dtype=bf16, unpacked_dtype=f32)
                         for i in range(2)], axis=0))
            else:
                xs = [x_v[rb, j, rows, :].astype(f32) for j in range(NJ)]
            for _ in range(2 * LNROLLX if roll else 0):
                xs = [pltpu.roll(x, 64, 1) for x in xs]
            t = xs[0]
            for j in range(1, NJ):
                t = t + xs[j]
            m = lane_sum(t, roll) * (1.0 / D)
            xc = [x - m for x in xs]
            t = xc[0] * xc[0]
            for j in range(1, NJ):
                t = t + xc[j] * xc[j]
            v = lane_sum(t, roll) * (1.0 / D)
            rs = lax.rsqrt(v + 1e-5)
            for j in range(NJ):
                y = xc[j] * rs
                for _ in range(2 * LNROLL2 if roll else 0):
                    y = pltpu.roll(y, 64, 1)
                if PK_X:
                    xn_v[rb, j, pl.ds(g * (LN_G // 2), LN_G // 2), :] = pltpu.pack_elementwise(
                        [y[:LN_G // 2], y[LN_G // 2:]], packed_dtype=bf16)
                else:
                    xn_v[rb, j, rows, :] = y.astype(bf16)

    def packed(ref):
        return pltpu.bitcast(ref.bitcast(u32)[...], bf16)

    def wide(ref, i):
        if PK_X:
            return jnp.concatenate([pltpu.bitcast(ref[i, j], bf16) for j in range(NJ)], axis=1)
        return jnp.concatenate([ref[i, j] for j in range(NJ)], axis=1)

    def ffn(rb, c, a=0, n=TF, first=False, waits=None, then=None):
        rows = pl.ds(pl.multiple_of(rb * TM, TM), TM)
        if not first and ACC_EARLY:
            y = acc_v[rows, :]
        xn = wide(xn_v, rb)
        j0 = c * (TF // 128) + a // 128
        if waits:
            wait(waits[0])
        w1 = jnp.concatenate([packed(w1_v.at[j0 + j]) for j in range(n // 128)], axis=1)
        g = jnp.dot(xn, w1, preferred_element_type=f32)
        if waits:
            wait(waits[1])
        w3 = jnp.concatenate([packed(w3_v.at[j0 + j]) for j in range(n // 128)], axis=1)
        u = jnp.dot(xn, w3, preferred_element_type=f32)
        hg = 0.5 * g
        t = hg * u
        h = t + t * jnp.tanh(hg)
        if waits:
            wait(waits[2])
            then()
        if n == TF:
            w2 = jnp.concatenate([packed(w2_v.at[c, j]) for j in range(NJ)], axis=1)
        else:
            w2 = jnp.concatenate([packed(w2_v.at[c, j, pl.ds(a, n)]) for j in range(NJ)], axis=1)
        d = jnp.dot(h.astype(bf16), w2, preferred_element_type=f32)
        acc_v[rows, :] = d if first else (y if ACC_EARLY else acc_v[rows, :]) + d

    def wt_prep(cb):
        sec, h0 = cb // 8, (cb % 8) * 4
        for kb in range(NJ):
            t = pltpu.bitcast(wqkv_v[pl.ds(kb * 128, 128), pl.ds(pl.multiple_of(cb * 128, 128), 128)].T, u32)
            for hh in range(4):
                wt_v[kb, pl.ds(sec * PITCH * 16 + h0 + hh, 16, stride=PITCH), :] = t[hh * 16:(hh + 1) * 16, :]

    def wo_prep(nb):
        t = wo_v.at[nb].bitcast(u32)[...]
        for h in range(H):
            wop_v[nb, pl.ds(h, 16, stride=PITCH), :] = t[h * 16:(h + 1) * 16, :]

    def qkv(rb):
        r0, m = pl.multiple_of(rb * TM, TM), TM
        xn = wide(xn_v, rb)
        for sec in range(3):
            wt = jnp.concatenate(
                [jnp.concatenate([pltpu.bitcast(wt_v[kb, pl.ds((sec * 16 + (dd ^ (PVROLL % 2 if sec == 2 else 0))) * PITCH, 32), :], bf16)
                                  for dd in range(16)], axis=0)
                 for kb in range(NJ)], axis=1)
            r = lax.dot_general(xn, wt, (((1,), (1,)), ((), ())), preferred_element_type=f32)
            for j in range(NJ):
                blk = r[:, j * 128:(j + 1) * 128]
                if sec == 0:
                    q_v[j, pl.ds(r0, m), :] = blk * (DH ** -0.5 * 1.4426950408889634) if PRESCALE else blk
                elif sec == 1:
                    k_v[j, pl.ds(r0 + PAD, m), :] = blk
                else:
                    v_v[j, pl.ds(r0 + PAD, m), :] = blk

    def attention(r0, rows, masked=False):
        c = DH ** -0.5 * 1.4426950408889634
        lane = lax.broadcasted_iota(jnp.int32, (16, 128), 1)
        even = (lane & 1) == 0
        lo = lane < 64
        sub = lax.broadcasted_iota(jnp.int32, (16, 128), 0)
        if PK_O:
            sub = (sub & 7) * 2 + (sub >> 3)

        def total(t):
            if TREE:
                return ((t[0] + t[1]) + (t[2] + t[3])) + ((t[4] + t[5]) + (t[6] + t[7]))
            p = t[0]
            for x in t[1:]:
                p = p + x
            return p

        for g in range(rows // 16):
            r = r0 + g * 16
            cache = {}

            def kw(ref, j, w, r=r, cache=cache):
                if PK_O:
                    return jnp.concatenate([ref[j, pl.ds(r + PAD - DIL * w + p, 8, stride=2), :] for p in range(2)], axis=0)
                if not KW24:
                    return ref[j, pl.ds(r + PAD - DIL * w, 16), :]
                key = (id(ref), j, w % 4)
                if key not in cache:
                    cache[key] = ref[j, pl.ds(r + PAD - DIL * (w % 4) - 8, 24), :]
                return cache[key][8:24] if w < 4 else cache[key][0:16]

            if PK_O:
                q = [jnp.concatenate([q_v[j, pl.ds(r + p, 8, stride=2), :] for p in range(2)], axis=0) for j in range(NJ)]
            else:
                q = [q_v[j, pl.ds(r, 16), :] for j in range(NJ)]
            if UPACK:
                P = [total([q[j] * kw(k_v, j, w) for j in range(NJ)]) for w in range(W)]
                for _ in range(QKROLL):
                    P = [pltpu.roll(p, 64, 1) for p in P]
                L = []
                for w in range(0, W, 2):
                    p = jnp.where(lo, P[w], P[w + 1]) + pltpu.roll(jnp.where(lo, P[w + 1], P[w]), 64, 1)
                    p = p + jnp.where(even, pltpu.roll(p, 127, 1), pltpu.roll(p, 1, 1))
                    if masked:
                        p = jnp.where(sub + r >= DIL * jnp.where(lo, w, w + 1), p, -1e30)
                    L.append(p)
                m = jnp.maximum(jnp.maximum(L[0], L[1]), jnp.maximum(L[2], L[3]))
                m = jnp.maximum(m, pltpu.roll(m, 64, 1))
                E = [jnp.exp2((l - m) * c) for l in L]
                den = (E[0] + E[1]) + (E[2] + E[3])
                den = den + pltpu.roll(den, 64, 1)
                inv = pl.reciprocal(den, approx=True)
                inv = inv * (2.0 - den * inv)
                A = []
                for e in E:
                    a = e * inv
                    b = pltpu.roll(a, 64, 1)
                    A += [jnp.where(lo, a, b), jnp.where(lo, b, a)]
            else:
                L = []
                for w in range(W):
                    p = total([q[j] * kw(k_v, j, w) for j in range(NJ)])
                    if ONESTAGE:
                        p = (p + pltpu.roll(p, 64, 1)) + jnp.where(
                            even, pltpu.roll(p, 127, 1) + pltpu.roll(p, 63, 1), pltpu.roll(p, 1, 1) + pltpu.roll(p, 65, 1))
                    elif NOROLL:
                        pass
                    else:
                        p = p + pltpu.roll(p, 64, 1)
                        p = p + jnp.where(even, pltpu.roll(p, 127, 1), pltpu.roll(p, 1, 1))
                    if masked and w > 0:
                        p = jnp.where(sub + r >= DIL * w, p, -1e30)
                    L.append(p)
                m = L[0]
                for w in range(1, W):
                    m = jnp.maximum(m, L[w])
                E = [jnp.exp2(l - m) if PRESCALE else jnp.exp2((l - m) * c) for l in L]
                den = total(E)
                if RECIP == 'newton':
                    inv = pl.reciprocal(den, approx=True)
                    inv = inv * (2.0 - den * inv)
                else:
                    inv = 1.0 / den
                A = E if NORM_O else [e * inv for e in E]
            for j in range(NJ):
                o = total([A[w] * kw(v_v, j, w) for w in range(W)])
                o = o * inv if NORM_O else o
                for _ in range(PVROLL):
                    o = pltpu.roll(o, 64, 1)
                if PK_O:
                    o_v[j, r // 16] = pltpu.pack_elementwise([o[:8], o[8:]], packed_dtype=bf16)
                else:
                    o_v[j, r // 16] = o.astype(bf16)

    def wo_mm(rb, j0=0, nj=NJ):
        rows = pl.ds(pl.multiple_of(rb * TM, TM), TM)
        cols = pl.ds(pl.multiple_of(j0 * 128, 128), nj * 128)
        y = acc_v[rows, cols]
        hg = 0.5 * y
        gate = hg + hg * jnp.tanh(hg)
        wop = jnp.concatenate(
            [jnp.concatenate([pltpu.bitcast(wop_v[j0 + nb, pl.ds(dd * PITCH, 32), :], bf16)
                              for dd in range(16)], axis=0)
             for nb in range(nj)], axis=1)
        if PK_O:
            o = jnp.concatenate([pltpu.bitcast(o_v[j, pl.ds(rb * (TM // 16), TM // 16)].reshape(TM // 2, 128), bf16)
                                 for j in range(NJ)], axis=1)
        else:
            o = jnp.concatenate([o_v[j, pl.ds(rb * (TM // 16), TM // 16)].reshape(TM, 128) for j in range(NJ)], axis=1)
        s = jnp.dot(o, wop, preferred_element_type=f32)
        for j in range(nj):
            c = slice(j * 128, (j + 1) * 128)
            out_v[rb, j0 + j] = (x_v[rb, j0 + j].astype(f32) + s[:, c] * gate[:, c]).astype(bf16)

    sub0 = cp_sub(0)
    start(cp_x(0))
    start(sub0[0])
    zpad = jnp.zeros((PAD, 128), f32)
    for j in range(NJ):
        k_v[j, pl.ds(0, PAD), :] = zpad
        v_v[j, pl.ds(0, PAD), :] = zpad
    wait(cp_x(0))
    start(sub0[1])
    start(sub0[2])
    layernorm(0)
    start(sum(cp_sub(1), []))

    ffn(0, 0, SUBS[0], SUBS[1] - SUBS[0], first=True, waits=sub0,
        then=lambda: start(sum(cp_sub(2), [])))
    wait(sum(cp_sub(1), []))
    start(cp_x(1))
    ffn(0, 0, SUBS[1], SUBS[2] - SUBS[1])
    wait(cp_x(1))
    wait(sum(cp_sub(2), []))
    start(cp_x(2))
    start(cp_x(3))
    ffn(0, 0, SUBS[2], SUBS[3] - SUBS[2])
    layernorm(1)
    wait(cp_x(2))
    wait(cp_x(3))
    start(cp_wo())
    start(cp_w(1))
    cp_qkv().start()
    one_ref[0] = 1
    one = one_ref[0]

    def block(f):
        if BLOCKS:
            lax.fori_loop(0, one, lambda i, c: (f(), c)[1], 0)
        else:
            f()

    for rb in range(1, NRB):
        def unit(rb=rb):
            ffn(rb, 0, first=True)
            if rb < NRB - 1:
                layernorm(rb + 1)
        if rb == NRB - 1 and WO_POS == 'end':
            wait(cp_wo())

            def unit(rb=rb):
                ffn(rb, 0, first=True)
                for nb in range(NJ):
                    wo_prep(nb)
        block(unit)

    cp_qkv().wait()
    if WO_POS != 'end':
        wait(cp_wo())
    wait(cp_w(1))
    start(cp_w(2))

    def l2(i, _):
        ffn(i, 1)
        for t in range(24 // NB):
            wt_prep(i * (24 // NB) + t)
        if WO_POS == 'l2':
            wo_prep(2 * i)
            wo_prep(2 * i + 1)
        return 0
    lax.fori_loop(0, NB, l2, 0)

    start(cp_w(3))

    def l3(i, _):
        qkv(i)
        if WO_POS == 'l3':
            wo_prep(2 * i)
            wo_prep(2 * i + 1)
        return 0
    lax.fori_loop(0, NB, l3, 0)

    wait(cp_w(2))
    wait(cp_w(3))

    def l4(i, _):
        ffn(i % NB, 2 + i // NB)
        attention(pl.multiple_of(i * (TB // 2), TB // 2), TB // 2)
        if WO_POS == 'l4':
            wo_prep(i)
        return 0
    lax.fori_loop(0, 2 * NB, l4, 0)

    attention(0, 16, masked=True)

    def l6(rb, _):
        wo_mm(rb)
        start(cp_out(rb))
        return 0
    lax.fori_loop(0, NRB - 1, l6, 0)

    def l7(hf, _):
        wo_mm(NRB - 1, hf * (NJ // 2), NJ // 2)
        start(cp_out(NRB - 1, hf * (NJ // 2), NJ // 2))
        return 0
    lax.fori_loop(0, 2, l7, 0)
    for rb in range(NRB):
        wait(cp_out(rb))


@jax.jit
def pallas_recurrent_scan__sliding_local_dilated__glu_gated_swiglu__prompt_kernel(
    A_x: jax.Array,
    A_wqkv: jax.Array,
    A_wo: jax.Array,
    B_x: jax.Array,
    B_w1: jax.Array,
    B_w3: jax.Array,
    B_w2: jax.Array,
):
    del B_x
    x = A_x.reshape(S, D)
    V = pltpu.VMEM
    DMA = pltpu.SemaphoreType.DMA
    out = pl.pallas_call(
        _kernel,
        out_shape=jax.ShapeDtypeStruct((S, D), bf16),
        in_specs=[pl.BlockSpec(memory_space=pl.ANY)] * 6,
        out_specs=pl.BlockSpec(memory_space=pl.ANY),
        scratch_shapes=[
            V((NRB, NJ, TM, 128), bf16),
            V((NRB, NJ, TM // 2, 128), u32) if PK_X else V((NRB, NJ, TM, 128), bf16),
            V((F // 128, D, 128), bf16), V((F // 128, D, 128), bf16), V((NC, NJ, TF, 128), bf16),
            V((D, 3 * D), bf16), V((NJ, 3 * 16 * PITCH, 128), u32),
            V((NJ, D, 128), bf16), V((NJ, 16 * PITCH, 128), u32),
            V((S, D), f32),
            V((NJ, S, 128), f32), V((NJ, S + PAD, 128), f32), V((NJ, S + PAD, 128), f32),
            V((NJ, S // 16, 8, 128), u32) if PK_O else V((NJ, S // 16, 16, 128), bf16), V((NRB, NJ, TM, 128), bf16),
            pltpu.SMEM((1,), jnp.int32),
            DMA((NRB,)), DMA((3, NC)), DMA((3, 3)), DMA(()), DMA(()), DMA((NRB,)),
        ],
        compiler_params=pltpu.CompilerParams(vmem_limit_bytes=120 * 1024 * 1024),
    )(x, A_wqkv, A_wo, B_w1, B_w3, B_w2)
    return out.reshape(1, S, D)
```

```python
import jax
import jax.numpy as jnp
from jax import lax
import jax.experimental.pallas as pl
import jax.experimental.pallas.tpu as pltpu

S, D, F = 2048, 1024, 3584
H, DH, W, DIL = 32, 32, 8, 2
TM = 512
NRB = S // TM
TF = 896
NC = F // TF
SUBS = (0, 256, 512, 896)
NJ = D // 128
PAD = 16
PITCH = 33
LN_G = 32
LN_NR = (0, 1, 3, 3)
ATT_ROWS = S // (2 * NRB)
f32, bf16, u32 = jnp.float32, jnp.bfloat16, jnp.uint32


def _kernel(x_hbm, wqkv_hbm, wo_hbm, w1_hbm, w3_hbm, w2_hbm, out_hbm,
            x_v, xn_v, w1_v, w3_v, w2_v, wqkv_v, wt_v, wo_v, wop_v, acc_v,
            q_v, k_v, v_v, o_v, out_v,
            sem_x, sem_w, sem_s, sem_qkv, sem_wo, sem_out):
    def cp_x(rb):
        return [pltpu.make_async_copy(x_hbm.at[pl.ds(rb * TM, TM), pl.ds(j * 128, 128)],
                                      x_v.at[rb, j], sem_x.at[rb]) for j in range(NJ)]

    def cp_cols(a, n, sems):
        groups = [[pltpu.make_async_copy(src.at[:, pl.ds(j * 128, 128)], dst.at[j], sem)
                   for j in range(a // 128, (a + n) // 128)]
                  for src, dst, sem in ((w1_hbm, w1_v, sems[0]), (w3_hbm, w3_v, sems[1]))]
        groups.append([pltpu.make_async_copy(w2_hbm.at[pl.ds(a, n), pl.ds(j * 128, 128)],
                                             w2_v.at[a // TF, j, pl.ds(a % TF, n)], sems[2])
                       for j in range(NJ)])
        return groups

    def cp_w(c):
        return sum(cp_cols(c * TF, TF, [sem_w.at[i, c] for i in range(3)]), [])

    def cp_sub(s):
        return cp_cols(SUBS[s], SUBS[s + 1] - SUBS[s], [sem_s.at[i, s] for i in range(3)])

    def cp_qkv():
        return [pltpu.make_async_copy(wqkv_hbm, wqkv_v, sem_qkv)]

    def cp_wo():
        return [pltpu.make_async_copy(wo_hbm.at[:, pl.ds(j * 128, 128)], wo_v.at[j], sem_wo)
                for j in range(NJ)]

    def cp_out(rb, j0=0, nj=NJ):
        r = pl.multiple_of(rb * TM, TM)
        return [pltpu.make_async_copy(
            out_v.at[rb, j0 + j],
            out_hbm.at[pl.ds(r, TM), pl.ds(pl.multiple_of((j0 + j) * 128, 128), 128)],
            sem_out.at[rb]) for j in range(nj)]

    def start(cps):
        for cp in cps:
            cp.start()

    def wait(cps):
        for cp in cps:
            cp.wait()

    def halves_swapped(t):
        return pltpu.roll(t, 64, 1)

    def lane_mean(t, nr):
        for sh in (64, 32, 16, 8, 4, 2, 1)[:nr]:
            t = t + pltpu.roll(t, sh, 1)
        return jnp.sum(t, axis=-1, keepdims=True) * (0.5 ** nr / D)

    def layernorm(rb):
        x32 = x_v.at[rb].bitcast(u32)
        half = LN_G // 2
        for g in range(TM // LN_G):
            rows = pl.ds(g * half, half)
            xs = []
            for j in range(NJ):
                w32 = x32[j, rows, :]
                xs.append(jnp.concatenate(
                    [pltpu.unpack_elementwise(w32, index=i, packed_dtype=bf16, unpacked_dtype=f32)
                     for i in range(2)], axis=0))
            t = xs[0]
            for j in range(1, NJ):
                t = t + xs[j]
            m = lane_mean(t, LN_NR[rb])
            xc = [x - m for x in xs]
            t = xc[0] * xc[0]
            for j in range(1, NJ):
                t = t + xc[j] * xc[j]
            rs = lax.rsqrt(lane_mean(t, LN_NR[rb]) + 1e-5)
            for j in range(NJ):
                y = xc[j] * rs
                xn_v[rb, j, rows, :] = pltpu.pack_elementwise([y[:half], y[half:]], packed_dtype=bf16)

    def packed(ref):
        return pltpu.bitcast(ref.bitcast(u32)[...], bf16)

    def xn_block(rb):
        return jnp.concatenate([pltpu.bitcast(xn_v[rb, j], bf16) for j in range(NJ)], axis=1)

    def ffn(rb, c, a=0, n=TF, first=False, hooks=None):
        rows = pl.ds(pl.multiple_of(rb * TM, TM), TM)
        xn = xn_block(rb)
        j0 = c * (TF // 128) + a // 128
        if hooks:
            hooks[0]()
        w1 = jnp.concatenate([packed(w1_v.at[j0 + j]) for j in range(n // 128)], axis=1)
        g = jnp.dot(xn, w1, preferred_element_type=f32)
        if hooks:
            hooks[1]()
        w3 = jnp.concatenate([packed(w3_v.at[j0 + j]) for j in range(n // 128)], axis=1)
        u = jnp.dot(xn, w3, preferred_element_type=f32)
        hg = 0.5 * g
        t = hg * u
        h = t + t * jnp.tanh(hg)
        if hooks:
            hooks[2]()
        if n == TF:
            w2 = jnp.concatenate([packed(w2_v.at[c, j]) for j in range(NJ)], axis=1)
        else:
            w2 = jnp.concatenate([packed(w2_v.at[c, j, pl.ds(a, n)]) for j in range(NJ)], axis=1)
        d = jnp.dot(h.astype(bf16), w2, preferred_element_type=f32)
        acc_v[rows, :] = d if first else acc_v[rows, :] + d

    def wt_prep(cb):
        sec, h0 = cb // 8, (cb % 8) * 4
        cols = pl.ds(pl.multiple_of(cb * 128, 128), 128)
        for kb in range(NJ):
            t = pltpu.bitcast(wqkv_v[pl.ds(kb * 128, 128), cols].T, u32)
            for hh in range(4):
                wt_v[kb, pl.ds(sec * PITCH * 16 + h0 + hh, 16, stride=PITCH), :] = t[hh * 16:(hh + 1) * 16, :]

    def wo_prep(nb):
        t = wo_v.at[nb].bitcast(u32)[...]
        for h in range(H):
            wop_v[nb, pl.ds(h, 16, stride=PITCH), :] = t[h * 16:(h + 1) * 16, :]

    def qkv(rb):
        r0 = pl.multiple_of(rb * TM, TM)
        xn = xn_block(rb)
        for sec in range(3):
            wt = jnp.concatenate(
                [jnp.concatenate(
                    [pltpu.bitcast(wt_v[kb, pl.ds((sec * 16 + (dd ^ (sec == 2))) * PITCH, 32), :], bf16)
                     for dd in range(16)], axis=0)
                 for kb in range(NJ)], axis=1)
            r = lax.dot_general(xn, wt, (((1,), (1,)), ((), ())), preferred_element_type=f32)
            dst, off = ((q_v, 0), (k_v, PAD), (v_v, PAD))[sec]
            for j in range(NJ):
                dst[j, pl.ds(r0 + off, TM), :] = r[:, j * 128:(j + 1) * 128]

    def attention(r0, rows, masked=False):
        c = DH ** -0.5 * 1.4426950408889634
        lane = lax.broadcasted_iota(jnp.int32, (16, 128), 1)
        even = (lane & 1) == 0
        lo = lane < 64
        sub = lax.broadcasted_iota(jnp.int32, (16, 128), 0)

        def total(terms):
            p = terms[0]
            for t in terms[1:]:
                p = p + t
            return p

        for g in range(rows // 16):
            r = r0 + g * 16
            cache = {}

            def shifted(ref, j, w, r=r, cache=cache):
                key = (id(ref), j, w % 4)
                if key not in cache:
                    cache[key] = ref[j, pl.ds(r + PAD - DIL * (w % 4) - 8, 24), :]
                return cache[key][8:24] if w < 4 else cache[key][0:16]

            q = [q_v[j, pl.ds(r, 16), :] for j in range(NJ)]
            part = [total([q[j] * shifted(k_v, j, w) for j in range(NJ)]) for w in range(W)]
            logits = []
            for w in range(0, W, 2):
                p = (jnp.where(lo, part[w], part[w + 1])
                     + halves_swapped(jnp.where(lo, part[w + 1], part[w])))
                p = p + jnp.where(even, pltpu.roll(p, 127, 1), pltpu.roll(p, 1, 1))
                if masked:
                    p = jnp.where(sub + r >= DIL * jnp.where(lo, w, w + 1), p, -1e30)
                logits.append(p)
            m = jnp.maximum(jnp.maximum(logits[0], logits[1]), jnp.maximum(logits[2], logits[3]))
            m = jnp.maximum(m, halves_swapped(m))
            e = [jnp.exp2((l - m) * c) for l in logits]
            den = (e[0] + e[1]) + (e[2] + e[3])
            den = den + halves_swapped(den)
            inv = pl.reciprocal(den, approx=True)
            inv = inv * (2.0 - den * inv)
            attn = []
            for t in e:
                a = t * inv
                b = halves_swapped(a)
                attn += [jnp.where(lo, a, b), jnp.where(lo, b, a)]
            for j in range(NJ):
                o = total([attn[w] * shifted(v_v, j, w) for w in range(W)])
                o = halves_swapped(halves_swapped(halves_swapped(o)))
                o_v[j, r // 16] = o.astype(bf16)

    def out_unit(rb, j0=0, nj=NJ):
        rows = pl.ds(pl.multiple_of(rb * TM, TM), TM)
        cols = pl.ds(pl.multiple_of(j0 * 128, 128), nj * 128)
        hy = 0.5 * acc_v[rows, cols]
        gate = hy + hy * jnp.tanh(hy)
        wop = jnp.concatenate(
            [jnp.concatenate([pltpu.bitcast(wop_v[j0 + nb, pl.ds(dd * PITCH, 32), :], bf16)
                              for dd in range(16)], axis=0)
             for nb in range(nj)], axis=1)
        o = jnp.concatenate([o_v[j, pl.ds(rb * (TM // 16), TM // 16)].reshape(TM, 128)
                             for j in range(NJ)], axis=1)
        s = jnp.dot(o, wop, preferred_element_type=f32)
        for j in range(nj):
            cj = slice(j * 128, (j + 1) * 128)
            out_v[rb, j0 + j] = (x_v[rb, j0 + j].astype(f32) + s[:, cj] * gate[:, cj]).astype(bf16)

    sub0, sub1, sub2 = cp_sub(0), sum(cp_sub(1), []), sum(cp_sub(2), [])
    start(cp_x(0))
    start(sub0[0])
    zpad = jnp.zeros((PAD, 128), f32)
    for j in range(NJ):
        k_v[j, pl.ds(0, PAD), :] = zpad
        v_v[j, pl.ds(0, PAD), :] = zpad
    wait(cp_x(0))
    start(sub0[1])
    start(sub0[2])
    layernorm(0)
    start(sub1)

    ffn(0, 0, SUBS[0], SUBS[1] - SUBS[0], first=True, hooks=(
        lambda: wait(sub0[0]),
        lambda: wait(sub0[1]),
        lambda: (wait(sub0[2]), start(sub2))))
    wait(sub1)
    start(cp_x(1))
    ffn(0, 0, SUBS[1], SUBS[2] - SUBS[1])
    wait(cp_x(1))
    wait(sub2)
    start(cp_x(2))
    start(cp_x(3))
    ffn(0, 0, SUBS[2], SUBS[3] - SUBS[2])
    layernorm(1)
    wait(cp_x(2))
    wait(cp_x(3))
    start(cp_wo())
    start(cp_w(1))
    start(cp_qkv())
    for rb in range(1, NRB):
        ffn(rb, 0, first=True)
        if rb < NRB - 1:
            layernorm(rb + 1)

    wait(cp_qkv())
    wait(cp_wo())
    wait(cp_w(1))
    start(cp_w(2))

    def ffn1_step(i, carry):
        ffn(i, 1)
        for t in range(3 * NJ // NRB):
            wt_prep(i * (3 * NJ // NRB) + t)
        for t in range(NJ // NRB):
            wo_prep(i * (NJ // NRB) + t)
        return carry
    lax.fori_loop(0, NRB, ffn1_step, 0)

    start(cp_w(3))

    def qkv_step(i, carry):
        qkv(i)
        return carry
    lax.fori_loop(0, NRB, qkv_step, 0)

    wait(cp_w(2))
    wait(cp_w(3))

    def ffn_att_step(i, carry):
        ffn(i % NRB, 2 + i // NRB)
        attention(pl.multiple_of(i * ATT_ROWS, ATT_ROWS), ATT_ROWS)
        return carry
    lax.fori_loop(0, 2 * NRB, ffn_att_step, 0)
    attention(0, 16, masked=True)

    for rb in range(NRB - 1):
        out_unit(rb)
        start(cp_out(rb))

    def last_step(hf, carry):
        out_unit(NRB - 1, hf * (NJ // 2), NJ // 2)
        start(cp_out(NRB - 1, hf * (NJ // 2), NJ // 2))
        return carry
    lax.fori_loop(0, 2, last_step, 0)
    for rb in range(NRB):
        wait(cp_out(rb))


@jax.jit
def pallas_recurrent_scan__sliding_local_dilated__glu_gated_swiglu__prompt_kernel(
    A_x: jax.Array,
    A_wqkv: jax.Array,
    A_wo: jax.Array,
    B_x: jax.Array,
    B_w1: jax.Array,
    B_w3: jax.Array,
    B_w2: jax.Array,
):
    del B_x
    vmem = pltpu.VMEM
    dma_sem = pltpu.SemaphoreType.DMA
    out = pl.pallas_call(
        _kernel,
        out_shape=jax.ShapeDtypeStruct((S, D), bf16),
        in_specs=[pl.BlockSpec(memory_space=pl.ANY)] * 6,
        out_specs=pl.BlockSpec(memory_space=pl.ANY),
        scratch_shapes=[
            vmem((NRB, NJ, TM, 128), bf16),
            vmem((NRB, NJ, TM // 2, 128), u32),
            vmem((F // 128, D, 128), bf16),
            vmem((F // 128, D, 128), bf16),
            vmem((NC, NJ, TF, 128), bf16),
            vmem((D, 3 * D), bf16),
            vmem((NJ, 3 * 16 * PITCH, 128), u32),
            vmem((NJ, D, 128), bf16),
            vmem((NJ, 16 * PITCH, 128), u32),
            vmem((S, D), f32),
            vmem((NJ, S, 128), f32),
            vmem((NJ, S + PAD, 128), f32),
            vmem((NJ, S + PAD, 128), f32),
            vmem((NJ, S // 16, 16, 128), bf16),
            vmem((NRB, NJ, TM, 128), bf16),
            dma_sem((NRB,)), dma_sem((3, NC)), dma_sem((3, len(SUBS) - 1)),
            dma_sem(()), dma_sem(()), dma_sem((NRB,)),
        ],
        compiler_params=pltpu.CompilerParams(vmem_limit_bytes=112 * 1024 * 1024),
    )(A_x.reshape(S, D), A_wqkv, A_wo, B_w1, B_w3, B_w2)
    return out.reshape(1, S, D)
```

```python
import jax
import jax.numpy as jnp
from jax import lax
import jax.experimental.pallas as pl
import jax.experimental.pallas.tpu as pltpu

S, D, F = 2048, 1024, 3584
H, DH, W, DIL = 32, 32, 8, 2
TM = 512
NRB = S // TM
TF = 896
NC = F // TF
SUBS = (0, 256, 512, 896)
NJ = D // 128
PAD = 16
PITCH = 33
LN_G = 32
LN_NR = (0, 1, 3, 3)
ATT_ROWS = S // (2 * NRB)
f32, bf16, u32 = jnp.float32, jnp.bfloat16, jnp.uint32


def _kernel(x_hbm, wqkv_hbm, wo_hbm, w1_hbm, w3_hbm, w2_hbm, out_hbm,
            x_v, xn_v, w1_v, w3_v, w2_v, wqkv_v, wt_v, wo_v, wop_v, acc_v,
            q_v, k_v, v_v, o_v, out_v,
            sem_x, sem_w, sem_s, sem_qkv, sem_wo, sem_out):
    def cp_x(rb):
        return [pltpu.make_async_copy(x_hbm.at[pl.ds(rb * TM, TM), pl.ds(j * 128, 128)],
                                      x_v.at[rb, j], sem_x.at[rb]) for j in range(NJ)]

    def cp_cols(a, n, sems):
        groups = [[pltpu.make_async_copy(src.at[:, pl.ds(j * 128, 128)], dst.at[j], sem)
                   for j in range(a // 128, (a + n) // 128)]
                  for src, dst, sem in ((w1_hbm, w1_v, sems[0]), (w3_hbm, w3_v, sems[1]))]
        groups.append([pltpu.make_async_copy(w2_hbm.at[pl.ds(a, n), pl.ds(j * 128, 128)],
                                             w2_v.at[a // TF, j, pl.ds(a % TF, n)], sems[2])
                       for j in range(NJ)])
        return groups

    def cp_w(c):
        return sum(cp_cols(c * TF, TF, [sem_w.at[i, c] for i in range(3)]), [])

    def cp_sub(s):
        return cp_cols(SUBS[s], SUBS[s + 1] - SUBS[s], [sem_s.at[i, s] for i in range(3)])

    def cp_qkv():
        return [pltpu.make_async_copy(wqkv_hbm, wqkv_v, sem_qkv)]

    def cp_wo():
        return [pltpu.make_async_copy(wo_hbm.at[:, pl.ds(j * 128, 128)], wo_v.at[j], sem_wo)
                for j in range(NJ)]

    def cp_out(rb, j0=0, nj=NJ):
        r = pl.multiple_of(rb * TM, TM)
        return [pltpu.make_async_copy(
            out_v.at[rb, j0 + j],
            out_hbm.at[pl.ds(r, TM), pl.ds(pl.multiple_of((j0 + j) * 128, 128), 128)],
            sem_out.at[rb]) for j in range(nj)]

    def start(cps):
        for cp in cps:
            cp.start()

    def wait(cps):
        for cp in cps:
            cp.wait()

    def halves_swapped(t):
        return pltpu.roll(t, 64, 1)

    def lane_mean(t, nr):
        for sh in (64, 32, 16, 8, 4, 2, 1)[:nr]:
            t = t + pltpu.roll(t, sh, 1)
        return jnp.sum(t, axis=-1, keepdims=True) * (0.5 ** nr / D)

    def layernorm(rb):
        for g in range(TM // LN_G):
            xs = [x_v[rb, j, pl.ds(g * LN_G, LN_G), :].astype(f32) for j in range(NJ)]
            t = xs[0]
            for j in range(1, NJ):
                t = t + xs[j]
            m = lane_mean(t, LN_NR[rb])
            xc = [x - m for x in xs]
            t = xc[0] * xc[0]
            for j in range(1, NJ):
                t = t + xc[j] * xc[j]
            rs = lax.rsqrt(lane_mean(t, LN_NR[rb]) + 1e-5)
            for j in range(NJ):
                xn_v[rb, j, pl.ds(g * LN_G, LN_G), :] = (xc[j] * rs).astype(bf16)

    def xn_block(rb):
        return jnp.concatenate([xn_v[rb, j] for j in range(NJ)], axis=1)

    def ffn(rb, c, a=0, n=TF, first=False, hooks=None):
        rows = pl.ds(pl.multiple_of(rb * TM, TM), TM)
        xn = xn_block(rb)
        j0 = c * (TF // 128) + a // 128
        if hooks:
            hooks[0]()
        w1 = jnp.concatenate([w1_v[j0 + j] for j in range(n // 128)], axis=1)
        g = jnp.dot(xn, w1, preferred_element_type=f32)
        if hooks:
            hooks[1]()
        w3 = jnp.concatenate([w3_v[j0 + j] for j in range(n // 128)], axis=1)
        u = jnp.dot(xn, w3, preferred_element_type=f32)
        hg = 0.5 * g
        t = hg * u
        h = t + t * jnp.tanh(hg)
        if hooks:
            hooks[2]()
        if n == TF:
            w2 = jnp.concatenate([w2_v[c, j] for j in range(NJ)], axis=1)
        else:
            w2 = jnp.concatenate([w2_v[c, j, pl.ds(a, n), :] for j in range(NJ)], axis=1)
        d = jnp.dot(h.astype(bf16), w2, preferred_element_type=f32)
        acc_v[rows, :] = d if first else acc_v[rows, :] + d

    def wt_prep(cb):
        sec, h0 = cb // 8, (cb % 8) * 4
        cols = pl.ds(pl.multiple_of(cb * 128, 128), 128)
        for kb in range(NJ):
            t = pltpu.bitcast(wqkv_v[pl.ds(kb * 128, 128), cols].T, u32)
            for hh in range(4):
                wt_v[kb, pl.ds(sec * PITCH * 16 + h0 + hh, 16, stride=PITCH), :] = t[hh * 16:(hh + 1) * 16, :]

    def wo_prep(nb):
        t = pltpu.bitcast(wo_v[nb], u32)
        for h in range(H):
            wop_v[nb, pl.ds(h, 16, stride=PITCH), :] = t[h * 16:(h + 1) * 16, :]

    def qkv(rb):
        r0 = pl.multiple_of(rb * TM, TM)
        xn = xn_block(rb)
        for sec in range(3):
            wt = jnp.concatenate(
                [jnp.concatenate(
                    [pltpu.bitcast(wt_v[kb, pl.ds((sec * 16 + (dd ^ (sec == 2))) * PITCH, 32), :], bf16)
                     for dd in range(16)], axis=0)
                 for kb in range(NJ)], axis=1)
            r = lax.dot_general(xn, wt, (((1,), (1,)), ((), ())), preferred_element_type=f32)
            dst, off = ((q_v, 0), (k_v, PAD), (v_v, PAD))[sec]
            for j in range(NJ):
                dst[j, pl.ds(r0 + off, TM), :] = r[:, j * 128:(j + 1) * 128]

    def attention(r0, rows, masked=False):
        c = DH ** -0.5 * 1.4426950408889634
        lane = lax.broadcasted_iota(jnp.int32, (16, 128), 1)
        even = (lane & 1) == 0
        lo = lane < 64
        sub = lax.broadcasted_iota(jnp.int32, (16, 128), 0)

        def total(terms):
            p = terms[0]
            for t in terms[1:]:
                p = p + t
            return p

        for g in range(rows // 16):
            r = r0 + g * 16
            cache = {}

            def shifted(ref, j, w, r=r, cache=cache):
                key = (id(ref), j, w % 4)
                if key not in cache:
                    cache[key] = ref[j, pl.ds(r + PAD - DIL * (w % 4) - 8, 24), :]
                return cache[key][8:24] if w < 4 else cache[key][0:16]

            q = [q_v[j, pl.ds(r, 16), :] for j in range(NJ)]
            part = [total([q[j] * shifted(k_v, j, w) for j in range(NJ)]) for w in range(W)]
            logits = []
            for w in range(0, W, 2):
                p = (jnp.where(lo, part[w], part[w + 1])
                     + halves_swapped(jnp.where(lo, part[w + 1], part[w])))
                p = p + jnp.where(even, pltpu.roll(p, 127, 1), pltpu.roll(p, 1, 1))
                if masked:
                    p = jnp.where(sub + r >= DIL * jnp.where(lo, w, w + 1), p, -1e30)
                logits.append(p)
            m = jnp.maximum(jnp.maximum(logits[0], logits[1]), jnp.maximum(logits[2], logits[3]))
            m = jnp.maximum(m, halves_swapped(m))
            e = [jnp.exp2((l - m) * c) for l in logits]
            den = (e[0] + e[1]) + (e[2] + e[3])
            den = den + halves_swapped(den)
            inv = pl.reciprocal(den, approx=True)
            inv = inv * (2.0 - den * inv)
            attn = []
            for t in e:
                a = t * inv
                b = halves_swapped(a)
                attn += [jnp.where(lo, a, b), jnp.where(lo, b, a)]
            for j in range(NJ):
                o = total([attn[w] * shifted(v_v, j, w) for w in range(W)])
                o = halves_swapped(halves_swapped(halves_swapped(o)))
                o_v[j, r // 16] = o.astype(bf16)

    def out_unit(rb, j0=0, nj=NJ):
        rows = pl.ds(pl.multiple_of(rb * TM, TM), TM)
        cols = pl.ds(pl.multiple_of(j0 * 128, 128), nj * 128)
        hy = 0.5 * acc_v[rows, cols]
        gate = hy + hy * jnp.tanh(hy)
        wop = jnp.concatenate(
            [jnp.concatenate([pltpu.bitcast(wop_v[j0 + nb, pl.ds(dd * PITCH, 32), :], bf16)
                              for dd in range(16)], axis=0)
             for nb in range(nj)], axis=1)
        o = jnp.concatenate([o_v[j, pl.ds(rb * (TM // 16), TM // 16)].reshape(TM, 128)
                             for j in range(NJ)], axis=1)
        s = jnp.dot(o, wop, preferred_element_type=f32)
        for j in range(nj):
            cj = slice(j * 128, (j + 1) * 128)
            out_v[rb, j0 + j] = (x_v[rb, j0 + j].astype(f32) + s[:, cj] * gate[:, cj]).astype(bf16)

    sub0, sub1, sub2 = cp_sub(0), sum(cp_sub(1), []), sum(cp_sub(2), [])
    start(cp_x(0))
    start(sub0[0])
    zpad = jnp.zeros((PAD, 128), f32)
    for j in range(NJ):
        k_v[j, pl.ds(0, PAD), :] = zpad
        v_v[j, pl.ds(0, PAD), :] = zpad
    wait(cp_x(0))
    start(sub0[1])
    start(sub0[2])
    layernorm(0)
    start(sub1)

    ffn(0, 0, SUBS[0], SUBS[1] - SUBS[0], first=True, hooks=(
        lambda: wait(sub0[0]),
        lambda: wait(sub0[1]),
        lambda: (wait(sub0[2]), start(sub2))))
    wait(sub1)
    start(cp_x(1))
    ffn(0, 0, SUBS[1], SUBS[2] - SUBS[1])
    wait(cp_x(1))
    wait(sub2)
    start(cp_x(2))
    start(cp_x(3))
    ffn(0, 0, SUBS[2], SUBS[3] - SUBS[2])
    layernorm(1)
    wait(cp_x(2))
    wait(cp_x(3))
    start(cp_wo())
    start(cp_w(1))
    start(cp_qkv())
    for rb in range(1, NRB):
        ffn(rb, 0, first=True)
        if rb < NRB - 1:
            layernorm(rb + 1)

    wait(cp_qkv())
    wait(cp_wo())
    wait(cp_w(1))
    start(cp_w(2))

    def ffn1_step(i, carry):
        ffn(i, 1)
        for t in range(3 * NJ // NRB):
            wt_prep(i * (3 * NJ // NRB) + t)
        for t in range(NJ // NRB):
            wo_prep(i * (NJ // NRB) + t)
        return carry
    lax.fori_loop(0, NRB, ffn1_step, 0)

    start(cp_w(3))

    def qkv_step(i, carry):
        qkv(i)
        return carry
    lax.fori_loop(0, NRB, qkv_step, 0)

    wait(cp_w(2))
    wait(cp_w(3))

    def ffn_att_step(i, carry):
        ffn(i % NRB, 2 + i // NRB)
        attention(pl.multiple_of(i * ATT_ROWS, ATT_ROWS), ATT_ROWS)
        return carry
    lax.fori_loop(0, 2 * NRB, ffn_att_step, 0)
    attention(0, 16, masked=True)

    for rb in range(NRB - 1):
        out_unit(rb)
        start(cp_out(rb))

    def last_step(hf, carry):
        out_unit(NRB - 1, hf * (NJ // 2), NJ // 2)
        start(cp_out(NRB - 1, hf * (NJ // 2), NJ // 2))
        return carry
    lax.fori_loop(0, 2, last_step, 0)
    for rb in range(NRB):
        wait(cp_out(rb))


@jax.jit
def pallas_recurrent_scan__sliding_local_dilated__glu_gated_swiglu__prompt_kernel(
    A_x: jax.Array,
    A_wqkv: jax.Array,
    A_wo: jax.Array,
    B_x: jax.Array,
    B_w1: jax.Array,
    B_w3: jax.Array,
    B_w2: jax.Array,
):
    del B_x
    vmem = pltpu.VMEM
    dma_sem = pltpu.SemaphoreType.DMA
    out = pl.pallas_call(
        _kernel,
        out_shape=jax.ShapeDtypeStruct((S, D), bf16),
        in_specs=[pl.BlockSpec(memory_space=pl.ANY)] * 6,
        out_specs=pl.BlockSpec(memory_space=pl.ANY),
        scratch_shapes=[
            vmem((NRB, NJ, TM, 128), bf16),
            vmem((NRB, NJ, TM, 128), bf16),
            vmem((F // 128, D, 128), bf16),
            vmem((F // 128, D, 128), bf16),
            vmem((NC, NJ, TF, 128), bf16),
            vmem((D, 3 * D), bf16),
            vmem((NJ, 3 * 16 * PITCH, 128), u32),
            vmem((NJ, D, 128), bf16),
            vmem((NJ, 16 * PITCH, 128), u32),
            vmem((S, D), f32),
            vmem((NJ, S, 128), f32),
            vmem((NJ, S + PAD, 128), f32),
            vmem((NJ, S + PAD, 128), f32),
            vmem((NJ, S // 16, 16, 128), bf16),
            vmem((NRB, NJ, TM, 128), bf16),
            dma_sem((NRB,)), dma_sem((3, NC)), dma_sem((3, len(SUBS) - 1)),
            dma_sem(()), dma_sem(()), dma_sem((NRB,)),
        ],
        compiler_params=pltpu.CompilerParams(vmem_limit_bytes=112 * 1024 * 1024),
    )(A_x.reshape(S, D), A_wqkv, A_wo, B_w1, B_w3, B_w2)
    return out.reshape(1, S, D)
```

```python
import jax
import jax.numpy as jnp
from jax import lax
import jax.experimental.pallas as pl
import jax.experimental.pallas.tpu as pltpu

S, D, F = 2048, 1024, 3584
H, DH, W, DIL = 32, 32, 8, 2
TM = 512
NRB = S // TM
TF = 896
NC = F // TF
SUBS = (0, 256, 512, 896)
NJ = D // 128
PAD = 16
PITCH = 33
LN_G = 32
LN_NR = (0, 2, 4, 4)
ATT_ROWS = S // (2 * NRB)
f32, bf16, u32 = jnp.float32, jnp.bfloat16, jnp.uint32


def _kernel(x_hbm, wqkv_hbm, wo_hbm, w1_hbm, w3_hbm, w2_hbm, out_hbm,
            x_v, xn_v, w1_v, w3_v, w2_v, wqkv_v, wt_v, wo_v, wop_v, acc_v,
            q_v, k_v, v_v, o_v, out_v,
            sem_x, sem_w, sem_s, sem_qkv, sem_wo, sem_out):
    def cp_x(rb):
        return [pltpu.make_async_copy(x_hbm.at[pl.ds(rb * TM, TM), pl.ds(j * 128, 128)],
                                      x_v.at[rb, j], sem_x.at[rb]) for j in range(NJ)]

    def cp_cols(a, n, sems):
        groups = [[pltpu.make_async_copy(src.at[:, pl.ds(j * 128, 128)], dst.at[j], sem)
                   for j in range(a // 128, (a + n) // 128)]
                  for src, dst, sem in ((w1_hbm, w1_v, sems[0]), (w3_hbm, w3_v, sems[1]))]
        groups.append([pltpu.make_async_copy(w2_hbm.at[pl.ds(a, n), pl.ds(j * 128, 128)],
                                             w2_v.at[a // TF, j, pl.ds(a % TF, n)], sems[2])
                       for j in range(NJ)])
        return groups

    def cp_w(c):
        return sum(cp_cols(c * TF, TF, [sem_w.at[i, c] for i in range(3)]), [])

    def cp_sub(s):
        return cp_cols(SUBS[s], SUBS[s + 1] - SUBS[s], [sem_s.at[i, s] for i in range(3)])

    def cp_qkv():
        return [pltpu.make_async_copy(wqkv_hbm, wqkv_v, sem_qkv)]

    def cp_wo():
        return [pltpu.make_async_copy(wo_hbm.at[:, pl.ds(j * 128, 128)], wo_v.at[j], sem_wo)
                for j in range(NJ)]

    def cp_out(rb, j0=0, nj=NJ):
        return [pltpu.make_async_copy(out_v.at[rb, j],
                                      out_hbm.at[pl.ds(rb * TM, TM), pl.ds(j * 128, 128)],
                                      sem_out.at[rb]) for j in range(j0, j0 + nj)]

    def start(cps):
        for cp in cps:
            cp.start()

    def wait(cps):
        for cp in cps:
            cp.wait()

    def halves_swapped(t):
        return pltpu.roll(t, 64, 1)

    def lane_mean(t, nr):
        for sh in (64, 32, 16, 8, 4, 2, 1)[:nr]:
            t = t + pltpu.roll(t, sh, 1)
        return jnp.sum(t, axis=-1, keepdims=True) * (0.5 ** nr / D)

    def layernorm(rb):
        for g in range(TM // LN_G):
            xs = [x_v[rb, j, pl.ds(g * LN_G, LN_G), :].astype(f32) for j in range(NJ)]
            t = xs[0]
            for j in range(1, NJ):
                t = t + xs[j]
            m = lane_mean(t, LN_NR[rb])
            xc = [x - m for x in xs]
            t = xc[0] * xc[0]
            for j in range(1, NJ):
                t = t + xc[j] * xc[j]
            rs = lax.rsqrt(lane_mean(t, LN_NR[rb]) + 1e-5)
            for j in range(NJ):
                xn_v[rb, j, pl.ds(g * LN_G, LN_G), :] = (xc[j] * rs).astype(bf16)

    def xn_block(rb):
        return jnp.concatenate([xn_v[rb, j] for j in range(NJ)], axis=1)

    def ffn(rb, c, a=0, n=TF, first=False, hooks=None):
        rows = pl.ds(pl.multiple_of(rb * TM, TM), TM)
        xn = xn_block(rb)
        j0 = c * (TF // 128) + a // 128
        if hooks:
            hooks[0]()
        w1 = jnp.concatenate([w1_v[j0 + j] for j in range(n // 128)], axis=1)
        g = jnp.dot(xn, w1, preferred_element_type=f32)
        if hooks:
            hooks[1]()
        w3 = jnp.concatenate([w3_v[j0 + j] for j in range(n // 128)], axis=1)
        u = jnp.dot(xn, w3, preferred_element_type=f32)
        hg = 0.5 * g
        t = hg * u
        h = t + t * jnp.tanh(hg)
        if hooks:
            hooks[2]()
        if n == TF:
            w2 = jnp.concatenate([w2_v[c, j] for j in range(NJ)], axis=1)
        else:
            w2 = jnp.concatenate([w2_v[c, j, pl.ds(a, n), :] for j in range(NJ)], axis=1)
        d = jnp.dot(h.astype(bf16), w2, preferred_element_type=f32)
        acc_v[rows, :] = d if first else acc_v[rows, :] + d

    def wt_prep(cb):
        sec, h0 = cb // 8, (cb % 8) * 4
        cols = pl.ds(pl.multiple_of(cb * 128, 128), 128)
        for kb in range(NJ):
            t = pltpu.bitcast(wqkv_v[pl.ds(kb * 128, 128), cols].T, u32)
            for hh in range(4):
                wt_v[kb, pl.ds(sec * PITCH * 16 + h0 + hh, 16, stride=PITCH), :] = t[hh * 16:(hh + 1) * 16, :]

    def wo_prep(nb):
        t = pltpu.bitcast(wo_v[nb], u32)
        for h in range(H):
            wop_v[nb, pl.ds(h, 16, stride=PITCH), :] = t[h * 16:(h + 1) * 16, :]

    def qkv(rb):
        r0 = pl.multiple_of(rb * TM, TM)
        xn = xn_block(rb)
        for sec in range(3):
            wt = jnp.concatenate(
                [jnp.concatenate(
                    [pltpu.bitcast(wt_v[kb, pl.ds((sec * 16 + (dd ^ (sec == 2))) * PITCH, 32), :], bf16)
                     for dd in range(16)], axis=0)
                 for kb in range(NJ)], axis=1)
            r = lax.dot_general(xn, wt, (((1,), (1,)), ((), ())), preferred_element_type=f32)
            dst, off = ((q_v, 0), (k_v, PAD), (v_v, PAD))[sec]
            for j in range(NJ):
                dst[j, pl.ds(r0 + off, TM), :] = r[:, j * 128:(j + 1) * 128]

    def attention(r0, rows, masked=False):
        c = DH ** -0.5 * 1.4426950408889634
        lane = lax.broadcasted_iota(jnp.int32, (16, 128), 1)
        even = (lane & 1) == 0
        lo = lane < 64
        sub = lax.broadcasted_iota(jnp.int32, (16, 128), 0)

        def total(terms):
            p = terms[0]
            for t in terms[1:]:
                p = p + t
            return p

        for g in range(rows // 16):
            r = r0 + g * 16
            cache = {}

            def shifted(ref, j, w, r=r, cache=cache):
                key = (id(ref), j, w % 4)
                if key not in cache:
                    cache[key] = ref[j, pl.ds(r + PAD - DIL * (w % 4) - 8, 24), :]
                return cache[key][8:24] if w < 4 else cache[key][0:16]

            q = [q_v[j, pl.ds(r, 16), :] for j in range(NJ)]
            part = [total([q[j] * shifted(k_v, j, w) for j in range(NJ)]) for w in range(W)]
            logits = []
            for w in range(0, W, 2):
                p = (jnp.where(lo, part[w], part[w + 1])
                     + halves_swapped(jnp.where(lo, part[w + 1], part[w])))
                p = p + jnp.where(even, pltpu.roll(p, 127, 1), pltpu.roll(p, 1, 1))
                if masked:
                    p = jnp.where(sub + r >= DIL * jnp.where(lo, w, w + 1), p, -1e30)
                logits.append(p)
            m = jnp.maximum(jnp.maximum(logits[0], logits[1]), jnp.maximum(logits[2], logits[3]))
            m = jnp.maximum(m, halves_swapped(m))
            e = [jnp.exp2((l - m) * c) for l in logits]
            den = (e[0] + e[1]) + (e[2] + e[3])
            den = den + halves_swapped(den)
            inv = pl.reciprocal(den, approx=True)
            inv = inv * (2.0 - den * inv)
            attn = []
            for t in e:
                a = t * inv
                b = halves_swapped(a)
                attn += [jnp.where(lo, a, b), jnp.where(lo, b, a)]
            for j in range(NJ):
                o = total([attn[w] * shifted(v_v, j, w) for w in range(W)])
                o = halves_swapped(halves_swapped(halves_swapped(o)))
                o_v[j, r // 16] = o.astype(bf16)

    def out_unit(rb, j0=0, nj=NJ):
        hy = 0.5 * acc_v[pl.ds(rb * TM, TM), pl.ds(j0 * 128, nj * 128)]
        gate = hy + hy * jnp.tanh(hy)
        wop = jnp.concatenate(
            [jnp.concatenate([pltpu.bitcast(wop_v[j0 + nb, pl.ds(dd * PITCH, 32), :], bf16)
                              for dd in range(16)], axis=0)
             for nb in range(nj)], axis=1)
        o = jnp.concatenate([o_v[j, pl.ds(rb * (TM // 16), TM // 16)].reshape(TM, 128)
                             for j in range(NJ)], axis=1)
        s = jnp.dot(o, wop, preferred_element_type=f32)
        for j in range(nj):
            cj = slice(j * 128, (j + 1) * 128)
            out_v[rb, j0 + j] = (x_v[rb, j0 + j].astype(f32) + s[:, cj] * gate[:, cj]).astype(bf16)

    sub0, sub1, sub2 = cp_sub(0), sum(cp_sub(1), []), sum(cp_sub(2), [])
    start(cp_x(0))
    zpad = jnp.zeros((PAD, 128), f32)
    for j in range(NJ):
        k_v[j, pl.ds(0, PAD), :] = zpad
        v_v[j, pl.ds(0, PAD), :] = zpad
    wait(cp_x(0))
    start(sub0[0])
    start(sub0[1])
    start(sub0[2])
    layernorm(0)
    start(sub1)

    ffn(0, 0, SUBS[0], SUBS[1] - SUBS[0], first=True, hooks=(
        lambda: wait(sub0[0]),
        lambda: wait(sub0[1]),
        lambda: (wait(sub0[2]), start(sub2))))
    wait(sub1)
    start(cp_x(1))
    ffn(0, 0, SUBS[1], SUBS[2] - SUBS[1])
    wait(cp_x(1))
    wait(sub2)
    start(cp_x(2))
    start(cp_x(3))
    ffn(0, 0, SUBS[2], SUBS[3] - SUBS[2])
    layernorm(1)
    wait(cp_x(2))
    wait(cp_x(3))
    start(cp_wo())
    start(cp_w(1))
    start(cp_qkv())
    for rb in range(1, NRB):
        ffn(rb, 0, first=True)
        if rb < NRB - 1:
            layernorm(rb + 1)

    wait(cp_qkv())
    wait(cp_wo())
    wait(cp_w(1))
    start(cp_w(2))

    def ffn1_step(i, carry):
        ffn(i, 1)
        for t in range(3 * NJ // NRB):
            wt_prep(i * (3 * NJ // NRB) + t)
        for t in range(NJ // NRB):
            wo_prep(i * (NJ // NRB) + t)
        return carry
    lax.fori_loop(0, NRB, ffn1_step, 0)

    start(cp_w(3))

    def qkv_step(i, carry):
        qkv(i)
        return carry
    lax.fori_loop(0, NRB, qkv_step, 0)

    wait(cp_w(2))
    wait(cp_w(3))

    def ffn_att_step(i, carry):
        ffn(i % NRB, 2 + i // NRB)
        attention(pl.multiple_of(i * ATT_ROWS, ATT_ROWS), ATT_ROWS)
        return carry
    lax.fori_loop(0, 2 * NRB, ffn_att_step, 0)

    for rb in (1, 2, 0):
        if rb == 2:
            attention(0, 16, masked=True)
        out_unit(rb)
        start(cp_out(rb))
    for j0, nj in ((0, 4), (4, 3), (7, 1)):
        out_unit(NRB - 1, j0, nj)
        start(cp_out(NRB - 1, j0, nj))
    for rb in range(NRB):
        wait(cp_out(rb))


@jax.jit
def pallas_recurrent_scan__sliding_local_dilated__glu_gated_swiglu__prompt_kernel(
    A_x: jax.Array,
    A_wqkv: jax.Array,
    A_wo: jax.Array,
    B_x: jax.Array,
    B_w1: jax.Array,
    B_w3: jax.Array,
    B_w2: jax.Array,
):
    del B_x
    vmem = pltpu.VMEM
    dma_sem = pltpu.SemaphoreType.DMA
    out = pl.pallas_call(
        _kernel,
        out_shape=jax.ShapeDtypeStruct((S, D), bf16),
        in_specs=[pl.BlockSpec(memory_space=pl.ANY)] * 6,
        out_specs=pl.BlockSpec(memory_space=pl.ANY),
        scratch_shapes=[
            vmem((NRB, NJ, TM, 128), bf16),
            vmem((NRB, NJ, TM, 128), bf16),
            vmem((F // 128, D, 128), bf16),
            vmem((F // 128, D, 128), bf16),
            vmem((NC, NJ, TF, 128), bf16),
            vmem((D, 3 * D), bf16),
            vmem((NJ, 3 * 16 * PITCH, 128), u32),
            vmem((NJ, D, 128), bf16),
            vmem((NJ, 16 * PITCH, 128), u32),
            vmem((S, D), f32),
            vmem((NJ, S, 128), f32),
            vmem((NJ, S + PAD, 128), f32),
            vmem((NJ, S + PAD, 128), f32),
            vmem((NJ, S // 16, 16, 128), bf16),
            vmem((NRB, NJ, TM, 128), bf16),
            dma_sem((NRB,)), dma_sem((3, NC)), dma_sem((3, len(SUBS) - 1)),
            dma_sem(()), dma_sem(()), dma_sem((NRB,)),
        ],
        compiler_params=pltpu.CompilerParams(vmem_limit_bytes=112 * 1024 * 1024),
    )(A_x.reshape(S, D), A_wqkv, A_wo, B_w1, B_w3, B_w2)
    return out.reshape(1, S, D)
```

```python
import jax
import jax.numpy as jnp
from jax import lax
import jax.experimental.pallas as pl
import jax.experimental.pallas.tpu as pltpu

S, D, F = 2048, 1024, 3584
H, DH, W, DIL = 32, 32, 8, 2
TM = 512
NRB = S // TM
TF = 896
NC = F // TF
SUBS = (0, 256, 512, 896)
NJ = D // 128
PAD = 16
PITCH = 33
LN_G = 32
LN_NR = (0, 2, 4, 4)
ATT_ROWS = S // (2 * NRB)
f32, bf16, u32 = jnp.float32, jnp.bfloat16, jnp.uint32


def _kernel(x_hbm, wqkv_hbm, wo_hbm, w1_hbm, w3_hbm, w2_hbm, out_hbm,
            x_v, xn_v, w1_v, w3_v, w2_v, wqkv_v, wt_v, wo_v, wop_v, acc_v,
            q_v, k_v, v_v, o_v, out_v,
            sem_x, sem_w, sem_s, sem_qkv, sem_wo, sem_out):
    def cp_x(rb):
        return [pltpu.make_async_copy(x_hbm.at[pl.ds(rb * TM, TM), pl.ds(j * 128, 128)],
                                      x_v.at[rb, j], sem_x.at[rb]) for j in range(NJ)]

    def cp_cols(a, n, sems):
        groups = [[pltpu.make_async_copy(src.at[:, pl.ds(j * 128, 128)], dst.at[j], sem)
                   for j in range(a // 128, (a + n) // 128)]
                  for src, dst, sem in ((w1_hbm, w1_v, sems[0]), (w3_hbm, w3_v, sems[1]))]
        groups.append([pltpu.make_async_copy(w2_hbm.at[pl.ds(a, n), pl.ds(j * 128, 128)],
                                             w2_v.at[a // TF, j, pl.ds(a % TF, n)], sems[2])
                       for j in range(NJ)])
        return groups

    def cp_w(c):
        return sum(cp_cols(c * TF, TF, [sem_w.at[i, c] for i in range(3)]), [])

    def cp_sub(s):
        return cp_cols(SUBS[s], SUBS[s + 1] - SUBS[s], [sem_s.at[i, s] for i in range(3)])

    def cp_qkv():
        return [pltpu.make_async_copy(wqkv_hbm, wqkv_v, sem_qkv)]

    def cp_wo():
        return [pltpu.make_async_copy(wo_hbm.at[:, pl.ds(j * 128, 128)], wo_v.at[j], sem_wo)
                for j in range(NJ)]

    def cp_out(rb, j0=0, nj=NJ):
        return [pltpu.make_async_copy(out_v.at[rb, j],
                                      out_hbm.at[pl.ds(rb * TM, TM), pl.ds(j * 128, 128)],
                                      sem_out.at[rb]) for j in range(j0, j0 + nj)]

    def start(cps):
        for cp in cps:
            cp.start()

    def wait(cps):
        for cp in cps:
            cp.wait()

    def halves_swapped(t):
        return pltpu.roll(t, 64, 1)

    def lane_mean(t, nr):
        for sh in (64, 32, 16, 8, 4, 2, 1)[:nr]:
            t = t + pltpu.roll(t, sh, 1)
        return jnp.sum(t, axis=-1, keepdims=True) * (0.5 ** nr / D)

    def layernorm(rb):
        for g in range(TM // LN_G):
            xs = [x_v[rb, j, pl.ds(g * LN_G, LN_G), :].astype(f32) for j in range(NJ)]
            t = xs[0]
            for j in range(1, NJ):
                t = t + xs[j]
            m = lane_mean(t, LN_NR[rb])
            xc = [x - m for x in xs]
            t = xc[0] * xc[0]
            for j in range(1, NJ):
                t = t + xc[j] * xc[j]
            rs = lax.rsqrt(lane_mean(t, LN_NR[rb]) + 1e-5)
            for j in range(NJ):
                xn_v[rb, j, pl.ds(g * LN_G, LN_G), :] = (xc[j] * rs).astype(bf16)

    def xn_block(rb):
        return jnp.concatenate([xn_v[rb, j] for j in range(NJ)], axis=1)

    def ffn(rb, c, a=0, n=TF, first=False, hooks=None):
        rows = pl.ds(pl.multiple_of(rb * TM, TM), TM)
        xn = xn_block(rb)
        j0 = c * (TF // 128) + a // 128
        if hooks:
            hooks[0]()
        w1 = jnp.concatenate([w1_v[j0 + j] for j in range(n // 128)], axis=1)
        g = jnp.dot(xn, w1, preferred_element_type=f32)
        if hooks:
            hooks[1]()
        w3 = jnp.concatenate([w3_v[j0 + j] for j in range(n // 128)], axis=1)
        u = jnp.dot(xn, w3, preferred_element_type=f32)
        hg = 0.5 * g
        t = hg * u
        h = t + t * jnp.tanh(hg)
        if hooks:
            hooks[2]()
        if n == TF:
            w2 = jnp.concatenate([w2_v[c, j] for j in range(NJ)], axis=1)
        else:
            w2 = jnp.concatenate([w2_v[c, j, pl.ds(a, n), :] for j in range(NJ)], axis=1)
        d = jnp.dot(h.astype(bf16), w2, preferred_element_type=f32)
        acc_v[rows, :] = d if first else acc_v[rows, :] + d

    def wt_prep(cb):
        sec, h0 = cb // 8, (cb % 8) * 4
        cols = pl.ds(pl.multiple_of(cb * 128, 128), 128)
        for kb in range(NJ):
            t = pltpu.bitcast(wqkv_v[pl.ds(kb * 128, 128), cols].T, u32)
            for hh in range(4):
                wt_v[kb, pl.ds(sec * PITCH * 16 + h0 + hh, 16, stride=PITCH), :] = t[hh * 16:(hh + 1) * 16, :]

    def wo_prep(nb):
        t = pltpu.bitcast(wo_v[nb], u32)
        for h in range(H):
            wop_v[nb, pl.ds(h, 16, stride=PITCH), :] = t[h * 16:(h + 1) * 16, :]

    def qkv(rb):
        r0 = pl.multiple_of(rb * TM, TM)
        xn = xn_block(rb)
        for sec in range(3):
            wt = jnp.concatenate(
                [jnp.concatenate(
                    [pltpu.bitcast(wt_v[kb, pl.ds((sec * 16 + (dd ^ (sec == 2))) * PITCH, 32), :], bf16)
                     for dd in range(16)], axis=0)
                 for kb in range(NJ)], axis=1)
            r = lax.dot_general(xn, wt, (((1,), (1,)), ((), ())), preferred_element_type=f32)
            dst, off = ((q_v, 0), (k_v, PAD), (v_v, PAD))[sec]
            for j in range(NJ):
                dst[j, pl.ds(r0 + off, TM), :] = r[:, j * 128:(j + 1) * 128]

    def attention(r0, rows, masked=False):
        c = DH ** -0.5 * 1.4426950408889634
        lane = lax.broadcasted_iota(jnp.int32, (16, 128), 1)
        even = (lane & 1) == 0
        lo = lane < 64
        sub = lax.broadcasted_iota(jnp.int32, (16, 128), 0)

        def total(terms):
            p = terms[0]
            for t in terms[1:]:
                p = p + t
            return p

        for g in range(rows // 16):
            r = r0 + g * 16
            cache = {}

            def shifted(name, j, w, r=r, cache=cache):
                key = (name, j, w % 4)
                if key not in cache:
                    ref = k_v if name == "k" else v_v
                    cache[key] = ref[j, pl.ds(r + PAD - DIL * (w % 4) - 8, 24), :]
                return cache[key][8:24] if w < 4 else cache[key][0:16]

            q = [q_v[j, pl.ds(r, 16), :] for j in range(NJ)]
            part = [total([q[j] * shifted("k", j, w) for j in range(NJ)]) for w in range(W)]
            logits = []
            for w in range(0, W, 2):
                p = (jnp.where(lo, part[w], part[w + 1])
                     + halves_swapped(jnp.where(lo, part[w + 1], part[w])))
                p = p + jnp.where(even, pltpu.roll(p, 127, 1), pltpu.roll(p, 1, 1))
                if masked:
                    p = jnp.where(sub + r >= DIL * jnp.where(lo, w, w + 1), p, -1e30)
                logits.append(p)
            m = jnp.maximum(jnp.maximum(logits[0], logits[1]), jnp.maximum(logits[2], logits[3]))
            m = jnp.maximum(m, halves_swapped(m))
            e = [jnp.exp2((l - m) * c) for l in logits]
            den = (e[0] + e[1]) + (e[2] + e[3])
            den = den + halves_swapped(den)
            inv = pl.reciprocal(den, approx=True)
            inv = inv * (2.0 - den * inv)
            attn = []
            for t in e:
                a = t * inv
                b = halves_swapped(a)
                attn += [jnp.where(lo, a, b), jnp.where(lo, b, a)]
            for j in range(NJ):
                o = total([attn[w] * shifted("v", j, w) for w in range(W)])
                o = halves_swapped(halves_swapped(halves_swapped(o)))
                o_v[j, r // 16] = o.astype(bf16)

    def out_unit(rb, j0=0, nj=NJ):
        hy = 0.5 * acc_v[pl.ds(rb * TM, TM), pl.ds(j0 * 128, nj * 128)]
        gate = hy + hy * jnp.tanh(hy)
        wop = jnp.concatenate(
            [jnp.concatenate([pltpu.bitcast(wop_v[j0 + nb, pl.ds(dd * PITCH, 32), :], bf16)
                              for dd in range(16)], axis=0)
             for nb in range(nj)], axis=1)
        o = jnp.concatenate([o_v[j, pl.ds(rb * (TM // 16), TM // 16)].reshape(TM, 128)
                             for j in range(NJ)], axis=1)
        s = jnp.dot(o, wop, preferred_element_type=f32)
        for j in range(nj):
            cj = slice(j * 128, (j + 1) * 128)
            out_v[rb, j0 + j] = (x_v[rb, j0 + j].astype(f32) + s[:, cj] * gate[:, cj]).astype(bf16)

    sub0, sub1, sub2 = cp_sub(0), sum(cp_sub(1), []), sum(cp_sub(2), [])
    start(cp_x(0))
    zpad = jnp.zeros((PAD, 128), f32)
    for j in range(NJ):
        k_v[j, pl.ds(0, PAD), :] = zpad
        v_v[j, pl.ds(0, PAD), :] = zpad
    wait(cp_x(0))
    start(sub0[0])
    start(sub0[1])
    start(sub0[2])
    layernorm(0)
    start(sub1)

    ffn(0, 0, SUBS[0], SUBS[1] - SUBS[0], first=True, hooks=(
        lambda: wait(sub0[0]),
        lambda: wait(sub0[1]),
        lambda: (wait(sub0[2]), start(sub2))))
    wait(sub1)
    start(cp_x(1))
    ffn(0, 0, SUBS[1], SUBS[2] - SUBS[1])
    wait(cp_x(1))
    wait(sub2)
    start(cp_x(2))
    start(cp_x(3))
    ffn(0, 0, SUBS[2], SUBS[3] - SUBS[2])
    layernorm(1)
    wait(cp_x(2))
    wait(cp_x(3))
    start(cp_wo())
    start(cp_w(1))
    start(cp_qkv())
    for rb in range(1, NRB):
        ffn(rb, 0, first=True)
        if rb < NRB - 1:
            layernorm(rb + 1)

    wait(cp_qkv())
    wait(cp_wo())
    wait(cp_w(1))
    start(cp_w(2))

    def ffn1_step(i, carry):
        ffn(i, 1)
        for t in range(3 * NJ // NRB):
            wt_prep(i * (3 * NJ // NRB) + t)
        for t in range(NJ // NRB):
            wo_prep(i * (NJ // NRB) + t)
        return carry
    lax.fori_loop(0, NRB, ffn1_step, 0)

    start(cp_w(3))

    def qkv_step(i, carry):
        qkv(i)
        return carry
    lax.fori_loop(0, NRB, qkv_step, 0)

    wait(cp_w(2))
    wait(cp_w(3))

    def ffn_att_step(i, carry):
        ffn(i % NRB, 2 + i // NRB)
        attention(pl.multiple_of(i * ATT_ROWS, ATT_ROWS), ATT_ROWS)
        return carry
    lax.fori_loop(0, 2 * NRB, ffn_att_step, 0)

    for rb in (1, 2, 0):
        if rb == 2:
            attention(0, 16, masked=True)
        out_unit(rb)
        start(cp_out(rb))
    for j0, nj in ((0, 4), (4, 3), (7, 1)):
        out_unit(NRB - 1, j0, nj)
        start(cp_out(NRB - 1, j0, nj))
    for rb in range(NRB):
        wait(cp_out(rb))


@jax.jit
def pallas_recurrent_scan__sliding_local_dilated__glu_gated_swiglu__prompt_kernel(
    A_x: jax.Array,
    A_wqkv: jax.Array,
    A_wo: jax.Array,
    B_x: jax.Array,
    B_w1: jax.Array,
    B_w3: jax.Array,
    B_w2: jax.Array,
):
    del B_x
    vmem = pltpu.VMEM
    dma_sem = pltpu.SemaphoreType.DMA
    out = pl.pallas_call(
        _kernel,
        out_shape=jax.ShapeDtypeStruct((S, D), bf16),
        in_specs=[pl.BlockSpec(memory_space=pl.ANY)] * 6,
        out_specs=pl.BlockSpec(memory_space=pl.ANY),
        scratch_shapes=[
            vmem((NRB, NJ, TM, 128), bf16),
            vmem((NRB, NJ, TM, 128), bf16),
            vmem((F // 128, D, 128), bf16),
            vmem((F // 128, D, 128), bf16),
            vmem((NC, NJ, TF, 128), bf16),
            vmem((D, 3 * D), bf16),
            vmem((NJ, 3 * 16 * PITCH, 128), u32),
            vmem((NJ, D, 128), bf16),
            vmem((NJ, 16 * PITCH, 128), u32),
            vmem((S, D), f32),
            vmem((NJ, S, 128), f32),
            vmem((NJ, S + PAD, 128), f32),
            vmem((NJ, S + PAD, 128), f32),
            vmem((NJ, S // 16, 16, 128), bf16),
            vmem((NRB, NJ, TM, 128), bf16),
            dma_sem((NRB,)), dma_sem((3, NC)), dma_sem((3, len(SUBS) - 1)),
            dma_sem(()), dma_sem(()), dma_sem((NRB,)),
        ],
        compiler_params=pltpu.CompilerParams(vmem_limit_bytes=112 * 1024 * 1024),
    )(A_x.reshape(S, D), A_wqkv, A_wo, B_w1, B_w3, B_w2)
    return out.reshape(1, S, D)
```
